```python
import os as _os
_os.environ.setdefault('JAX_PLATFORMS', 'cpu')
import jax
import jax.numpy as jnp

def _softmax(x, axis=-1):
    return jax.nn.softmax(x, axis=axis)

def _gelu(x):
    return jax.nn.gelu(x, approximate=True)

def _silu(x):
    return jax.nn.silu(x)

def _sigmoid(x):
    return jax.nn.sigmoid(x)

def _layernorm(x, axis=-1, eps=1e-05):
    m = jnp.mean(x, axis=axis, keepdims=True)
    v = jnp.var(x, axis=axis, keepdims=True)
    return (x - m) / jnp.sqrt(v + eps)

def _scatter_add(tgt, idx, src, axis=0):
    return tgt.at[idx].add(src)

def _segment_sum(src, seg, n):
    return jax.ops.segment_sum(src, seg, n)

class _Rng:

    def __init__(self, key):
        self._k = key

    def _next(self):
        self._k, sub = jax.random.split(self._k)
        return sub

    def normal(self, shape):
        return jax.random.normal(self._next(), shape, dtype=jnp.bfloat16)

    def randint(self, lo, hi, shape):
        return jax.random.randint(self._next(), shape, lo, hi, dtype=jnp.int32)

    def uniform(self, shape, lo=0.0, hi=1.0):
        return jax.random.uniform(self._next(), shape, jnp.bfloat16, lo, hi)

    def permutation(self, n):
        return jax.random.permutation(self._next(), n)
kernel_name = 'sequential_preLN__memory_aug_recurrent_mem_tr__swiglu_ffn__prompt'

def setup_inputs():
    _rng = _Rng(jax.random.key(int.from_bytes(__import__("os").urandom(4), "little")))
    _w = lambda a: (lambda t: t.astype(jnp.bfloat16) if jnp.issubdtype(t.dtype, jnp.floating) else t)(jnp.asarray(a))

    def _A_setup():
        B, S, Dm = (1, 2048, 640)
        H, Dh = (32, 192)
        M, seg = (8, 32)
        seg = min(seg, S)
        S = S // seg * seg
        return {'x': _w((lambda *s: _rng.normal(s) * 0.05)(B, S, Dm)), 'mem0': _w((lambda *s: _rng.normal(s) * 0.1)(B, M, Dm)), 'Wq': _w((lambda *s: _rng.normal(s) * 1.6)(Dm, H, Dh) * Dm ** (-0.5)), 'Wk': _w((lambda *s: _rng.normal(s) * 1.6)(Dm, H, Dh) * Dm ** (-0.5)), 'Wv': _w((lambda *s: _rng.normal(s) * 0.1)(Dm, H, Dh) * Dm ** (-0.5)), 'Wo': _w((lambda *s: _rng.normal(s) * 0.1)(H, Dh, Dm) * (H * Dh) ** (-0.5)), 'seg_len': seg}
    _A_in = _A_setup()

    def _B_setup():
        B, S, D, F = (1, 2048, 640, 1536)
        return {'x': _w((lambda *s: _rng.normal(s) * 0.05)(B, S, D)), 'w_gate': _w((lambda *s: _rng.normal(s) * 0.05)(D, F)), 'w_up': _w((lambda *s: _rng.normal(s) * 0.05)(D, F)), 'w_down': _w((lambda *s: _rng.normal(s) * 0.05)(F, D))}
    _B_in = _B_setup()
    return {'A_x': _A_in['x'], 'A_mem0': _A_in['mem0'], 'A_Wq': _A_in['Wq'], 'A_Wk': _A_in['Wk'], 'A_Wv': _A_in['Wv'], 'A_Wo': _A_in['Wo'], 'A_seg_len': _A_in['seg_len'], 'B_x': _B_in['x'], 'B_w_gate': _B_in['w_gate'], 'B_w_up': _B_in['w_up'], 'B_w_down': _B_in['w_down']}

def reference(A_x, A_mem0, A_Wq, A_Wk, A_Wv, A_Wo, A_seg_len, B_x, B_w_gate, B_w_up, B_w_down):

    def _A_ref(x, mem0, Wq, Wk, Wv, Wo, seg_len):
        B, S, Dm = x.shape
        H, Dh = (Wq.shape[1], Wq.shape[2])
        M = mem0.shape[1]
        scale = Dh ** (-0.5)
        n_seg = S // seg_len
        L = M + seg_len
        idx = jnp.arange(L)
        mask = (idx[:, None] < M) | (idx[:, None] >= idx[None, :])
        mem = mem0
        outs = []
        for s in range(n_seg):
            xs = x[:, s * seg_len:(s + 1) * seg_len, :].copy()
            h = jnp.concatenate([mem, xs], axis=1)
            q = jnp.einsum('btd,dhe->bhte', h, Wq)
            k = jnp.einsum('btd,dhe->bhte', h, Wk)
            v = jnp.einsum('btd,dhe->bhte', h, Wv)
            scores = jnp.einsum('bhqe,bhke->bhqk', q, k) * scale
            scores = jnp.where(mask[None, None], scores, -1000000000.0)
            p = _softmax(scores, axis=-1)
            o = jnp.einsum('bhqk,bhke->bhqe', p, v)
            o = jnp.einsum('bhte,hed->btd', o, Wo)
            mem = o[:, :M, :].copy()
            outs.append(o[:, M:, :])
        return jnp.concatenate(outs, axis=1)

    def _B_ref(x, w_gate, w_up, w_down):
        g = _silu(x @ w_gate)
        u = x @ w_up
        return g * u @ w_down
    x = A_x
    h = x + _A_ref(_layernorm(x, axis=-1), A_mem0, A_Wq, A_Wk, A_Wv, A_Wo, A_seg_len)
    h2 = h + _B_ref(_layernorm(h, axis=-1), B_w_gate, B_w_up, B_w_down)
    return h2
```

```python
import functools

import jax
import jax.numpy as jnp
import jax.experimental.pallas as pl
import jax.experimental.pallas.tpu as pltpu

F32 = jnp.float32
BF16 = jnp.bfloat16

_NT = (((1,), (1,)), ((), ()))


def _ln(x):
    m = jnp.mean(x, axis=-1, keepdims=True)
    xc = x - m
    v = jnp.mean(xc * xc, axis=-1, keepdims=True)
    return xc * jax.lax.rsqrt(v + 1e-05)


def _make_kernel(S, D, H, DH, M, SEG, F):
    NSEG = S // SEG
    NP = H // 2
    PW = 2 * DH
    RP = SEG - M
    RD = SEG - RP
    L = M + SEG
    ND = NSEG * RD
    NSLOT = 6
    FB = 256
    SEG_PER_FB = FB // SEG
    NFB = S // FB
    scale = float(DH) ** -0.5

    def kernel(x_hbm, mem_hbm, wq_hbm, wk_hbm, wv_hbm, wo_hbm, wg_hbm, wu_hbm, wd_hbm,
               out_hbm,
               x_v, mem_v, stage, wqkv, wo_v, wg_v, wu_v, wd_v,
               xd_v, qd, kd2, vd2, h_v, out_v, o_v,
               sem_in, sem_stage, sem_out):
        w_hbm = (wq_hbm, wk_hbm, wv_hbm)

        def stage_copy(p, which, slot):
            return pltpu.make_async_copy(
                w_hbm[which].at[pl.ds(p * PW, PW), :], stage.at[slot], sem_stage.at[slot])

        cp_x = pltpu.make_async_copy(x_hbm, x_v, sem_in.at[0])
        cp_mem = pltpu.make_async_copy(mem_hbm, mem_v, sem_in.at[1])
        cp_wo = pltpu.make_async_copy(wo_hbm, wo_v, sem_in.at[2])
        cp_wg = pltpu.make_async_copy(wg_hbm, wg_v, sem_in.at[3])
        cp_wu = pltpu.make_async_copy(wu_hbm, wu_v, sem_in.at[4])
        cp_wd = pltpu.make_async_copy(wd_hbm, wd_v, sem_in.at[5])

        cp_x.start()
        cp_mem.start()
        for p in range(2):
            for which in range(3):
                stage_copy(p, which, p * 3 + which).start()

        cp_x.wait()
        xd = x_v[:, RP:SEG, :].astype(F32).reshape(ND, D)
        xd_v[...] = _ln(xd).astype(BF16)

        lane_p = jax.lax.broadcasted_iota(jnp.int32, (1, 1, PW), 2)
        is_a3 = lane_p < DH

        def pro_body(p, carry):
            col = pl.multiple_of(p * PW, 128)
            for which in range(3):
                slot = (p % 2) * 3 + which
                stage_copy(p, which, slot).wait()
                w = stage[slot]
                y = jax.lax.dot_general(xd_v[...], w, _NT, preferred_element_type=F32)
                y3 = y.reshape(NSEG, RD, PW)
                if which == 0:
                    qd[:, :, pl.ds(col, PW)] = y3.astype(BF16)
                else:
                    ya = jnp.where(is_a3, y3, 0.0)
                    yb = jnp.where(is_a3, 0.0, y3)
                    dst = kd2 if which == 1 else vd2
                    dst[:, :, pl.ds(col, PW)] = jnp.concatenate([ya, yb], axis=1).astype(BF16)
                wqkv[p, :, which * PW:(which + 1) * PW] = w.T

                @pl.when(p + 2 < NP)
                def _():
                    stage_copy(p + 2, which, slot).start()

            @pl.when(p == NP - 3)
            def _():
                cp_wo.start()
                cp_wg.start()
                cp_wu.start()
                cp_wd.start()
            return carry

        jax.lax.fori_loop(0, NP, pro_body, 0)
        cp_mem.wait()
        cp_wo.wait()

        NK = 2 * L
        R1 = M + RP
        row = jax.lax.broadcasted_iota(jnp.int32, (L, NK), 0)
        lane = jax.lax.broadcasted_iota(jnp.int32, (L, NK), 1)
        in_main = lane < 2 * R1
        is_a = (lane < R1) | ((lane >= 2 * R1) & (lane < 2 * R1 + RD))
        key = jnp.where(in_main,
                        jnp.where(lane < R1, lane, lane - R1),
                        jnp.where(is_a, lane - R1, lane - R1 - RD))
        causal = (row < M) | (row >= key)
        lane2 = jax.lax.broadcasted_iota(jnp.int32, (1, PW), 1)
        is_a2 = lane2 < DH

        def seg_body(s, m):
            xs = x_v[s, 0:RP, :].astype(F32)
            l1 = jnp.concatenate([m, _ln(xs)], axis=0).astype(BF16)

            def stage_a(p):
                c0, c1 = p * PW, (p + 1) * PW
                y = jnp.dot(l1, wqkv[p], preferred_element_type=F32)
                q = y[:, 0:PW]
                k = y[:, PW:2 * PW]
                v = y[:, 2 * PW:3 * PW]
                qf = jnp.concatenate([q.astype(BF16), qd[s, :, c0:c1]], axis=0)
                kbd = jnp.concatenate([jnp.where(is_a2, k, 0.0).astype(BF16),
                                       jnp.where(is_a2, 0.0, k).astype(BF16),
                                       kd2[s, :, c0:c1]], axis=0)
                vbd = jnp.concatenate([jnp.where(is_a2, v, 0.0).astype(BF16),
                                       jnp.where(is_a2, 0.0, v).astype(BF16),
                                       vd2[s, :, c0:c1]], axis=0)
                return qf, kbd, vbd

            def stage_b(qf, kbd):
                sc = jax.lax.dot_general(qf, kbd, _NT, preferred_element_type=F32) * scale
                sc = jnp.where(causal, sc, -1000000000.0)
                ma = jnp.max(jnp.where(is_a, sc, -jnp.inf), axis=1, keepdims=True)
                mb = jnp.max(jnp.where(is_a, -jnp.inf, sc), axis=1, keepdims=True)
                e = jnp.exp(sc - jnp.where(is_a, ma, mb))
                sa = jnp.sum(jnp.where(is_a, e, 0.0), axis=1, keepdims=True)
                sb = jnp.sum(jnp.where(is_a, 0.0, e), axis=1, keepdims=True)
                return (e / jnp.where(is_a, sa, sb)).astype(BF16)

            def stage_d(p, pm, vbd):
                c0, c1 = p * PW, (p + 1) * PW
                o = jnp.dot(pm, vbd, preferred_element_type=F32).astype(BF16)
                qd[s, :, c0:c1] = o[R1:L]
                o_v[:, c0:c1] = o[0:R1]

            def stage_e(p0, p1):
                c0, c1 = p0 * PW, p1 * PW
                return jnp.dot(o_v[:, c0:c1], wo_v[c0:c1, :], preferred_element_type=F32)

            abuf = {}
            pbuf = {}
            for t in range(NP):
                abuf[t] = stage_a(t)
                if t >= 1:
                    pbuf[t - 1] = stage_b(abuf[t - 1][0], abuf[t - 1][1])
                if t >= 2:
                    stage_d(t - 2, pbuf[t - 2], abuf[t - 2][2])
            acc = stage_e(0, 2)
            pbuf[NP - 1] = stage_b(abuf[NP - 1][0], abuf[NP - 1][1])
            stage_d(NP - 2, pbuf[NP - 2], abuf[NP - 2][2])
            acc = acc + stage_e(2, 7)
            stage_d(NP - 1, pbuf[NP - 1], abuf[NP - 1][2])
            acc = acc + stage_e(7, NP - 1)
            acc = acc + stage_e(NP - 1, NP)
            h_v[s, 0:RP, :] = xs + acc[M:R1]
            return acc[0:M]

        jax.lax.fori_loop(0, NSEG, seg_body, mem_v[...].astype(F32))

        od = qd[...].reshape(ND, H * DH)
        a = jnp.dot(od, wo_v[...], preferred_element_type=F32)
        h_v[:, RP:SEG, :] = x_v[:, RP:SEG, :].astype(F32) + a.reshape(NSEG, RD, D)

        cp_wg.wait()
        cp_wu.wait()
        cp_wd.wait()

        def out_copy(b):
            seg0 = pl.multiple_of(b * SEG_PER_FB, SEG_PER_FB)
            return pltpu.make_async_copy(
                out_v.at[pl.ds(seg0, SEG_PER_FB)], out_hbm.at[pl.ds(seg0, SEG_PER_FB)],
                sem_out.at[b])

        def ffn_body(b, carry):
            seg0 = pl.multiple_of(b * SEG_PER_FB, SEG_PER_FB)
            h = h_v[pl.ds(seg0, SEG_PER_FB)].reshape(FB, D)
            hn = _ln(h).astype(BF16)
            g = jnp.dot(hn, wg_v[...], preferred_element_type=F32)
            u = jnp.dot(hn, wu_v[...], preferred_element_type=F32)
            act = (g * jax.nn.sigmoid(g) * u).astype(BF16)
            y = h + jnp.dot(act, wd_v[...], preferred_element_type=F32)
            out_v[pl.ds(seg0, SEG_PER_FB)] = y.astype(BF16).reshape(SEG_PER_FB, SEG, D)
            out_copy(b).start()
            return carry

        jax.lax.fori_loop(0, NFB, ffn_body, 0)
        for b in range(NFB):
            out_copy(b).wait()

    scratch = [
        pltpu.VMEM((NSEG, SEG, D), BF16),
        pltpu.VMEM((M, D), BF16),
        pltpu.VMEM((NSLOT, PW, D), BF16),
        pltpu.VMEM((NP, D, 3 * PW), BF16),
        pltpu.VMEM((H * DH, D), BF16),
        pltpu.VMEM((D, F), BF16),
        pltpu.VMEM((D, F), BF16),
        pltpu.VMEM((F, D), BF16),
        pltpu.VMEM((ND, D), BF16),
        pltpu.VMEM((NSEG, RD, H * DH), BF16),
        pltpu.VMEM((NSEG, 2 * RD, H * DH), BF16),
        pltpu.VMEM((NSEG, 2 * RD, H * DH), BF16),
        pltpu.VMEM((NSEG, SEG, D), F32),
        pltpu.VMEM((NSEG, SEG, D), BF16),
        pltpu.VMEM((M + RP, H * DH), BF16),
        pltpu.SemaphoreType.DMA((6,)),
        pltpu.SemaphoreType.DMA((NSLOT,)),
        pltpu.SemaphoreType.DMA((NFB,)),
    ]
    return kernel, scratch


@functools.partial(jax.jit, static_argnames=("seg",))
def _impl(A_x, A_mem0, A_Wq, A_Wk, A_Wv, A_Wo, B_w_gate, B_w_up, B_w_down, *, seg):
    B, S, D = A_x.shape
    _, H, DH = A_Wq.shape
    M = A_mem0.shape[1]
    F = B_w_gate.shape[1]
    assert B == 1 and S % seg == 0 and seg == 32 and M == 8
    nseg = S // seg

    kernel, scratch = _make_kernel(S, D, H, DH, M, seg, F)

    x3 = A_x.reshape(nseg, seg, D)
    mem = A_mem0.reshape(M, D)
    wqT = jnp.transpose(A_Wq, (1, 2, 0)).reshape(H * DH, D)
    wkT = jnp.transpose(A_Wk, (1, 2, 0)).reshape(H * DH, D)
    wvT = jnp.transpose(A_Wv, (1, 2, 0)).reshape(H * DH, D)
    wo = A_Wo.reshape(H * DH, D)

    out = pl.pallas_call(
        kernel,
        out_shape=jax.ShapeDtypeStruct((nseg, seg, D), A_x.dtype),
        in_specs=[pl.BlockSpec(memory_space=pl.ANY)] * 9,
        out_specs=pl.BlockSpec(memory_space=pl.ANY),
        scratch_shapes=scratch,
        compiler_params=pltpu.CompilerParams(vmem_limit_bytes=110 * 1024 * 1024),
    )(x3, mem, wqT, wkT, wvT, wo, B_w_gate, B_w_up, B_w_down)
    return out.reshape(B, S, D)


def pallas_sequential_preLN__memory_aug_recurrent_mem_tr__swiglu_ffn__prompt_kernel(
    A_x,
    A_mem0,
    A_Wq,
    A_Wk,
    A_Wv,
    A_Wo,
    A_seg_len,
    B_x,
    B_w_gate,
    B_w_up,
    B_w_down,
):
    seg = A_seg_len if isinstance(A_seg_len, int) else 32
    return _impl(A_x, A_mem0, A_Wq, A_Wk, A_Wv, A_Wo, B_w_gate, B_w_up, B_w_down, seg=seg)
```

```python
import functools

import jax
import jax.numpy as jnp
import jax.experimental.pallas as pl
import jax.experimental.pallas.tpu as pltpu

F32 = jnp.float32
BF16 = jnp.bfloat16

_NT = (((1,), (1,)), ((), ()))
_NEG = -1000000000.0


def _ln(x):
    m = jnp.mean(x, axis=-1, keepdims=True)
    xc = x - m
    v = jnp.mean(xc * xc, axis=-1, keepdims=True)
    return xc * jax.lax.rsqrt(v + 1e-05)


def _pair_softmax(sc, visible, own_a, own_b):
    sc = jnp.where(visible, sc, _NEG)
    sa_ = jnp.where(own_a, sc, -jnp.inf)
    sb_ = jnp.where(own_b, sc, -jnp.inf)
    ma = jnp.max(sa_, axis=1, keepdims=True)
    mb = jnp.max(sb_, axis=1, keepdims=True)
    e = jnp.exp(jnp.where(own_a, sa_ - ma, sb_ - mb))
    da = jnp.sum(jnp.where(own_a, e, 0.0), axis=1, keepdims=True)
    db = jnp.sum(jnp.where(own_a, 0.0, e), axis=1, keepdims=True)
    return (e / jnp.where(own_a, da, db)).astype(BF16)


def _make_kernel(S, D, H, DH, M, SEG, F):
    NSEG = S // SEG
    NP = H // 2
    PW = 2 * DH
    RD = M
    RP = SEG - RD
    R1 = M + RP
    ND = NSEG * RD
    NSLOT = 3
    SPP = NSEG // NP
    NJ = NSEG // 2
    FW = 128
    FC = F // FW
    FR = 2 * SEG
    SCHED_A = (((0, 2), (2, 5), (5, 8), (8, 16)), (1, 2))
    SCHED_B = (tuple((p, p + 1) for p in range(NP)), (2, 4))
    SCHED_B0 = (tuple((p, p + 1) for p in range(NP)), (4, 5))
    QKF = 0.7
    DA_QK_AT = tuple(1 + int(p * QKF) for p in range(NP))
    DA_PV_AT = tuple(max(p, DA_QK_AT[p] + 3) for p in range(NP))
    scale = float(DH) ** -0.5
    LAG_B = 1
    LAG_D = 2
    E_CHUNKS = ((0, 3), (3, 6), (6, 9), (9, 12), (12, 16))

    def kernel(x_hbm, mem_hbm, wq_hbm, wk_hbm, wv_hbm, wo_hbm, wg_hbm, wu_hbm, wd_hbm,
               out_hbm,
               x_v, mem_v, stage, wqkv, wo_v, wg_v, wu_v, wd_v,
               xd_raw, xd_v, qd, kd2, vd2, km2, vm2, h_v, out_v, o_v, hb_v, act_v,
               sem_in, sem_stage, sem_wo, sem_out):
        w_hbm = (wq_hbm, wk_hbm, wv_hbm)

        def stage_copies(p, slot):
            cps = [pltpu.make_async_copy(
                w_hbm[which].at[pl.ds(p * PW, PW), :],
                stage.at[slot, pl.ds(which * PW, PW), :],
                sem_stage.at[slot, which]) for which in range(3)]
            cps.append(pltpu.make_async_copy(
                x_hbm.at[pl.ds(p * SPP, SPP)], x_v.at[pl.ds(p * SPP, SPP)],
                sem_stage.at[slot, 3]))
            return cps

        def wo_copy(p):
            return pltpu.make_async_copy(
                wo_hbm.at[pl.ds(p * PW, PW), :], wo_v.at[pl.ds(p * PW, PW), :], sem_wo.at[p])

        cp_xd = pltpu.make_async_copy(x_hbm.at[:, pl.ds(0, RD), :], xd_raw, sem_in.at[0])
        cp_mem = pltpu.make_async_copy(mem_hbm, mem_v, sem_in.at[1])
        cp_wg = pltpu.make_async_copy(wg_hbm, wg_v, sem_in.at[2])
        cp_wu = pltpu.make_async_copy(wu_hbm, wu_v, sem_in.at[3])
        cp_wd = pltpu.make_async_copy(wd_hbm, wd_v, sem_in.at[4])

        cp_xd.start()
        for cp in stage_copies(0, 0):
            cp.start()

        cp_xd.wait()
        cp_mem.start()
        for cp in stage_copies(1, 1):
            cp.start()
        xd = xd_raw[...].astype(F32).reshape(ND, D)
        xd_v[...] = _ln(xd).astype(BF16)

        lane_p = jax.lax.broadcasted_iota(jnp.int32, (1, 1, PW), 2)
        is_a3 = lane_p < DH

        def pro_body(p, carry):
            slot = p % NSLOT
            for cp in stage_copies(p, slot):
                cp.wait()

            @pl.when(p + 2 < NP)
            def _():
                for cp in stage_copies(p + 2, (p + 2) % NSLOT):
                    cp.start()

            wo_copy(p).start()

            col = pl.multiple_of(p * PW, 128)
            w = stage[slot]
            y = jax.lax.dot_general(xd_v[...], w, _NT, preferred_element_type=F32)
            y3 = y.reshape(NSEG, RD, 3 * PW)
            qd[:, :, pl.ds(col, PW)] = y3[:, :, 0:PW].astype(BF16)
            for which, dst in ((1, kd2), (2, vd2)):
                yw = y3[:, :, which * PW:(which + 1) * PW]
                ya = jnp.where(is_a3, yw, 0.0)
                yb = jnp.where(is_a3, 0.0, yw)
                dst[:, :, pl.ds(col, PW)] = jnp.concatenate([ya, yb], axis=1).astype(BF16)
            wqkv[p] = w.T
            seg0 = pl.multiple_of(p * SPP, SPP)
            h_v[pl.ds(seg0, SPP), RD:SEG, :] = _ln(x_v[pl.ds(seg0, SPP), RD:SEG, :].astype(F32))
            return carry

        jax.lax.fori_loop(0, NP, pro_body, 0)
        cp_mem.wait()
        for p in range(NP):
            wo_copy(p).wait()
        cp_wg.start()
        cp_wu.start()
        cp_wd.start()

        NK = 2 * (R1 + RD)
        row = jax.lax.broadcasted_iota(jnp.int32, (R1, NK), 0)
        lane = jax.lax.broadcasted_iota(jnp.int32, (R1, NK), 1)
        c_own_a = (lane < R1) | ((lane >= 2 * R1) & (lane < 2 * R1 + RD))
        c_own_b = jnp.logical_not(c_own_a)
        c_vis = (row < M) | (lane >= 2 * R1) | ((lane & (R1 - 1)) <= row)
        NKD = 2 * 2 * (M + RD)
        rowd = jax.lax.broadcasted_iota(jnp.int32, (2 * RD, NKD), 0)
        laned = jax.lax.broadcasted_iota(jnp.int32, (2 * RD, NKD), 1)
        same_seg = (rowd >= RD) == (laned >= NKD // 2)
        d_is_a = (laned & RD) == 0
        d_own_a = same_seg & d_is_a
        d_own_b = same_seg & jnp.logical_not(d_is_a)
        d_vis = ((laned & (2 * M)) == 0) | ((laned & (RD - 1)) <= (rowd & (RD - 1)))
        lane2 = jax.lax.broadcasted_iota(jnp.int32, (1, PW), 1)
        is_a2 = lane2 < DH

        def seg_step(s, half, m, xn, extras, erows, sched):
            l1 = jnp.concatenate([m, xn], axis=0).astype(BF16)

            def blockdiag(t, d2_ref, m2_ref, c0, c1):
                ta = jnp.where(is_a2, t, 0.0)
                tb = jnp.where(is_a2, 0.0, t)
                m2_ref[half, :, c0:c1] = jnp.concatenate(
                    [ta[0:M], tb[0:M]], axis=0).astype(BF16)
                return jnp.concatenate(
                    [ta.astype(BF16), tb.astype(BF16), d2_ref[s, :, c0:c1]], axis=0)

            def stage_a(p):
                c0, c1 = p * PW, (p + 1) * PW
                y = jnp.dot(l1, wqkv[p], preferred_element_type=F32)
                qf = y[:, 0:PW].astype(BF16)
                kbd = blockdiag(y[:, PW:2 * PW], kd2, km2, c0, c1)
                vbd = blockdiag(y[:, 2 * PW:3 * PW], vd2, vm2, c0, c1)
                return qf, kbd, vbd

            def stage_b(qf, kbd):
                sc = jax.lax.dot_general(qf, kbd, _NT, preferred_element_type=F32) * scale
                return _pair_softmax(sc, c_vis, c_own_a, c_own_b)

            def stage_d(p, pm, vbd):
                c0, c1 = p * PW, (p + 1) * PW
                o_v[0:R1, c0:c1] = jnp.dot(pm, vbd, preferred_element_type=F32).astype(BF16)

            def stage_e(p0, p1):
                c0, c1 = p0 * PW, p1 * PW
                return jnp.dot(o_v[0:erows, c0:c1], wo_v[c0:c1, :], preferred_element_type=F32)

            def run(key):
                for fn in extras.get(key, ()):
                    fn()

            e_chunks, d_tail = sched
            pos_b = {p: p + 1 for p in range(NP)}
            pos_d = {p: p + 2 for p in range(NP - 2)}
            pos_d[NP - 2], pos_d[NP - 1] = NP + d_tail[0], NP + d_tail[1]
            abuf = {}
            pbuf = {}
            acc = None
            for t in range(NP + len(e_chunks)):
                if t < NP:
                    abuf[t] = stage_a(t)
                else:
                    part = stage_e(*e_chunks[t - NP])
                    acc = part if acc is None else acc + part
                run(t)
                for p in range(NP):
                    if pos_b[p] == t:
                        pbuf[p] = stage_b(abuf[p][0], abuf[p][1])
                for p in range(NP):
                    if pos_d[p] == t:
                        stage_d(p, pbuf[p], abuf[p][2])
                run(("post", t))
            h_v[s, RD:SEG, :] = x_v[s, RD:SEG, :].astype(F32) + acc[M:R1]
            return acc

        def da_qk(s0, p):
            c0, c1 = p * PW, (p + 1) * PW
            q = jnp.concatenate([qd[s0, :, c0:c1], qd[s0 + 1, :, c0:c1]], axis=0)
            k = jnp.concatenate([km2[0, :, c0:c1], kd2[s0, :, c0:c1],
                                 km2[1, :, c0:c1], kd2[s0 + 1, :, c0:c1]], axis=0)
            sc = jax.lax.dot_general(q, k, _NT, preferred_element_type=F32) * scale
            return _pair_softmax(sc, d_vis, d_own_a, d_own_b)

        def da_pv(s0, p, pm):
            c0, c1 = p * PW, (p + 1) * PW
            v = jnp.concatenate([vm2[0, :, c0:c1], vd2[s0, :, c0:c1],
                                 vm2[1, :, c0:c1], vd2[s0 + 1, :, c0:c1]], axis=0)
            o_v[R1:R1 + 2 * RD, c0:c1] = jnp.dot(pm, v, preferred_element_type=F32).astype(BF16)

        def out_copy(s0, n, k):
            return pltpu.make_async_copy(
                out_v.at[pl.ds(s0, n)], out_hbm.at[pl.ds(s0, n)], sem_out.at[k])

        def main_body(j, m, first=False):
            s0 = 0 if first else pl.multiple_of(2 * j, 2)
            xn0 = h_v[s0, RD:SEG, :]
            xn1 = h_v[s0 + 1, RD:SEG, :]
            pieces = []
            if not first:
                s1 = pl.multiple_of((j - 1) * 2, 2)
                s2 = pl.multiple_of(jnp.maximum(j - 2, 0) * 2, 2)
                hb_v[...] = jnp.concatenate(
                    [h_v[s2, 0:RD, :], h_v[s2 + 1, 0:RD, :],
                     h_v[s1, RD:SEG, :], h_v[s1 + 1, RD:SEG, :]], axis=0)
                hn = _ln(hb_v[...]).astype(BF16)

                gbuf = {}

                def gate(c):
                    gbuf[c] = jnp.dot(hn, wg_v[:, c * FW:(c + 1) * FW], preferred_element_type=F32)

                def up(c):
                    u = jnp.dot(hn, wu_v[:, c * FW:(c + 1) * FW], preferred_element_type=F32)
                    g = gbuf[c]
                    act_v[:, c * FW:(c + 1) * FW] = (g * jax.nn.sigmoid(g) * u).astype(BF16)

                def down(n, half):
                    n0, n1 = n * 128, (n + 1) * 128
                    f0, f1 = half * (F // 2), (half + 1) * (F // 2)
                    y = hb_v[:, n0:n1] + jnp.dot(act_v[:, f0:f1], wd_v[f0:f1, n0:n1],
                                                 preferred_element_type=F32)
                    if half == 0:
                        hb_v[:, n0:n1] = y
                    else:
                        y = y.astype(BF16)
                        out_v[s2, 0:RD, n0:n1] = y[0:RD]
                        out_v[s2 + 1, 0:RD, n0:n1] = y[RD:2 * RD]
                        out_v[s1, RD:SEG, n0:n1] = y[2 * RD:2 * RD + RP]
                        out_v[s1 + 1, RD:SEG, n0:n1] = y[2 * RD + RP:FR]

                for c in range(FC):
                    pieces += [functools.partial(gate, c), functools.partial(up, c)]
                for half in range(2):
                    pieces += [functools.partial(down, n, half) for n in range(D // 128)]
            na = NP
            nb = len(pieces) - 2 * NP

            extras = {} if first else {t + 1: [pieces[t]] for t in range(na)}
            acc = seg_step(s0, 0, m, xn0, extras, R1, SCHED_A)
            for fn in pieces[na:na + nb]:
                fn()

            pd = {}

            def qk(p):
                pd[p] = da_qk(s0, p)

            def pv(p):
                da_pv(s0, p, pd[p])

            extras = {} if first else {t + 1: [pieces[na + nb + t]] for t in range(NP)}
            for p in range(NP):
                extras.setdefault(("post", NP + DA_QK_AT[p]), []).append(functools.partial(qk, p))
                extras.setdefault(("post", NP + DA_PV_AT[p]), []).append(functools.partial(pv, p))
            acc = seg_step(s0 + 1, 1, acc[0:M], xn1, extras, R1 if first else R1 + 2 * RD,
                           SCHED_B0 if first else SCHED_B)
            if not first:
                h_v[s1, 0:RD, :] = x_v[s1, 0:RD, :].astype(F32) + acc[R1:R1 + RD]
                h_v[s1 + 1, 0:RD, :] = x_v[s1 + 1, 0:RD, :].astype(F32) + acc[R1 + RD:R1 + 2 * RD]

                @pl.when(j >= 2)
                def _():
                    out_copy(s2, 2, j - 2).start()
            return acc[0:M]

        h_v[0:2, 0:RD, :] = jnp.zeros((2, RD, D), F32)
        m1 = main_body(0, mem_v[...].astype(F32), first=True)
        cp_wg.wait()
        cp_wu.wait()
        cp_wd.wait()
        jax.lax.fori_loop(1, NJ, main_body, m1)

        sl = NSEG - 2
        a = jnp.dot(o_v[R1:R1 + 2 * RD, :], wo_v[...], preferred_element_type=F32)
        hl0 = x_v[sl, 0:RD, :].astype(F32) + a[0:RD]
        hl1 = x_v[sl + 1, 0:RD, :].astype(F32) + a[RD:2 * RD]
        h = jnp.concatenate([h_v[sl - 2, 0:RD, :], h_v[sl - 1, 0:RD, :],
                             hl0, h_v[sl, RD:SEG, :], hl1, h_v[sl + 1, RD:SEG, :]], axis=0)
        hn = _ln(h).astype(BF16)
        g = jnp.dot(hn, wg_v[...], preferred_element_type=F32)
        u = jnp.dot(hn, wu_v[...], preferred_element_type=F32)
        act = (g * jax.nn.sigmoid(g) * u).astype(BF16)
        y = (h + jnp.dot(act, wd_v[...], preferred_element_type=F32)).astype(BF16)
        out_v[sl - 2, 0:RD, :] = y[0:RD]
        out_v[sl - 1, 0:RD, :] = y[RD:2 * RD]
        out_v[sl] = y[2 * RD:2 * RD + SEG]
        out_v[sl + 1] = y[2 * RD + SEG:2 * RD + 2 * SEG]
        out_copy(sl - 2, 4, NJ - 2).start()

        for j in range(2, NJ):
            out_copy(2 * j - 4, 2, j - 2).wait()
        out_copy(sl - 2, 4, NJ - 2).wait()

    scratch = [
        pltpu.VMEM((NSEG, SEG, D), BF16),
        pltpu.VMEM((M, D), BF16),
        pltpu.VMEM((NSLOT, 3 * PW, D), BF16),
        pltpu.VMEM((NP, D, 3 * PW), BF16),
        pltpu.VMEM((H * DH, D), BF16),
        pltpu.VMEM((D, F), BF16),
        pltpu.VMEM((D, F), BF16),
        pltpu.VMEM((F, D), BF16),
        pltpu.VMEM((NSEG, RD, D), BF16),
        pltpu.VMEM((ND, D), BF16),
        pltpu.VMEM((NSEG, RD, H * DH), BF16),
        pltpu.VMEM((NSEG, 2 * RD, H * DH), BF16),
        pltpu.VMEM((NSEG, 2 * RD, H * DH), BF16),
        pltpu.VMEM((2, 2 * M, H * DH), BF16),
        pltpu.VMEM((2, 2 * M, H * DH), BF16),
        pltpu.VMEM((NSEG, SEG, D), F32),
        pltpu.VMEM((NSEG, SEG, D), BF16),
        pltpu.VMEM((R1 + 2 * RD, H * DH), BF16),
        pltpu.VMEM((FR, D), F32),
        pltpu.VMEM((FR, F), BF16),
        pltpu.SemaphoreType.DMA((5,)),
        pltpu.SemaphoreType.DMA((NSLOT, 4)),
        pltpu.SemaphoreType.DMA((NP,)),
        pltpu.SemaphoreType.DMA((NJ,)),
    ]
    return kernel, scratch


@functools.partial(jax.jit, static_argnames=("seg",))
def _impl(A_x, A_mem0, A_Wq, A_Wk, A_Wv, A_Wo, B_w_gate, B_w_up, B_w_down, *, seg):
    B, S, D = A_x.shape
    _, H, DH = A_Wq.shape
    M = A_mem0.shape[1]
    F = B_w_gate.shape[1]
    assert B == 1 and S % seg == 0 and seg == 32 and M == 8
    nseg = S // seg

    kernel, scratch = _make_kernel(S, D, H, DH, M, seg, F)

    x3 = A_x.reshape(nseg, seg, D)
    mem = A_mem0.reshape(M, D)
    wqT = jnp.transpose(A_Wq, (1, 2, 0)).reshape(H * DH, D)
    wkT = jnp.transpose(A_Wk, (1, 2, 0)).reshape(H * DH, D)
    wvT = jnp.transpose(A_Wv, (1, 2, 0)).reshape(H * DH, D)
    wo = A_Wo.reshape(H * DH, D)

    out = pl.pallas_call(
        kernel,
        out_shape=jax.ShapeDtypeStruct((nseg, seg, D), A_x.dtype),
        in_specs=[pl.BlockSpec(memory_space=pl.ANY)] * 9,
        out_specs=pl.BlockSpec(memory_space=pl.ANY),
        scratch_shapes=scratch,
        compiler_params=pltpu.CompilerParams(vmem_limit_bytes=110 * 1024 * 1024, disable_bounds_checks=True, disable_semaphore_checks=True),
    )(x3, mem, wqT, wkT, wvT, wo, B_w_gate, B_w_up, B_w_down)
    return out.reshape(B, S, D)


def pallas_sequential_preLN__memory_aug_recurrent_mem_tr__swiglu_ffn__prompt_kernel(
    A_x,
    A_mem0,
    A_Wq,
    A_Wk,
    A_Wv,
    A_Wo,
    A_seg_len,
    B_x,
    B_w_gate,
    B_w_up,
    B_w_down,
):
    seg = A_seg_len if isinstance(A_seg_len, int) else 32
    return _impl(A_x, A_mem0, A_Wq, A_Wk, A_Wv, A_Wo, B_w_gate, B_w_up, B_w_down, seg=seg)
```

```python
import functools

import jax
import jax.numpy as jnp
import jax.experimental.pallas as pl
import jax.experimental.pallas.tpu as pltpu

F32 = jnp.float32
BF16 = jnp.bfloat16

_NT = (((1,), (1,)), ((), ()))
_NEG = -1000000000.0


def _ln(x):
    m = jnp.mean(x, axis=-1, keepdims=True)
    xc = x - m
    v = jnp.mean(xc * xc, axis=-1, keepdims=True)
    return xc * jax.lax.rsqrt(v + 1e-05)


def _pair_softmax(sc, visible, own_a, own_b):
    sc = jnp.where(visible, sc, _NEG)
    sa_ = jnp.where(own_a, sc, -jnp.inf)
    sb_ = jnp.where(own_b, sc, -jnp.inf)
    ma = jnp.max(sa_, axis=1, keepdims=True)
    mb = jnp.max(sb_, axis=1, keepdims=True)
    e = jnp.exp(jnp.where(own_a, sa_ - ma, sb_ - mb))
    da = jnp.sum(jnp.where(own_a, e, 0.0), axis=1, keepdims=True)
    db = jnp.sum(jnp.where(own_a, 0.0, e), axis=1, keepdims=True)
    return (e / jnp.where(own_a, da, db)).astype(BF16)


def _make_kernel(S, D, H, DH, M, SEG, F):
    NSEG = S // SEG
    NP = H // 2
    PW = 2 * DH
    RD = M
    RP = SEG - RD
    R1 = M + RP
    ND = NSEG * RD
    NSLOT = 3
    PRB = 4
    SPP = NSEG // NP
    NJ = NSEG // 2
    FW = 128
    FC = F // FW
    FR = 2 * SEG
    SCHED_A = (((0, 2), (2, 5), (5, 8), (8, 16)), (1, 2))
    SCHED_B = (tuple((p, p + 1) for p in range(NP)), (2, 4))
    SCHED_B0 = (tuple((p, p + 1) for p in range(NP)), (4, 5))
    QKF = 0.7
    DA_QK_AT = tuple(1 + int(p * QKF) for p in range(NP))
    DA_PV_AT = tuple(max(p, DA_QK_AT[p] + 3) for p in range(NP))
    scale = float(DH) ** -0.5
    LAG_B = 1
    LAG_D = 2
    E_CHUNKS = ((0, 3), (3, 6), (6, 9), (9, 12), (12, 16))

    def kernel(x_hbm, mem_hbm, wq_hbm, wk_hbm, wv_hbm, wo_hbm, wg_hbm, wu_hbm, wd_hbm,
               out_hbm,
               x_v, mem_v, stage, wqkv, wo_v, wg_v, wu_v, wd_v,
               xd_raw, xd_v, qd, kd, vd, km2, vm2, h_v, out_v, o_v, hb_v, act_v,
               sem_in, sem_stage, sem_out):
        w_hbm = (wq_hbm, wk_hbm, wv_hbm, wo_hbm)

        def w_copy(p, which):
            slot = p % NSLOT
            return pltpu.make_async_copy(
                w_hbm[which].at[pl.ds(p * PW, PW), :],
                stage.at[slot, pl.ds(which * PW, PW), :], sem_stage.at[slot, which])

        def qkv_copies(p):
            return [w_copy(p, which) for which in range(3)]

        def ox_copies(p):
            return [w_copy(p, 3), pltpu.make_async_copy(
                x_hbm.at[pl.ds(p * SPP, SPP)], x_v.at[pl.ds(p * SPP, SPP)],
                sem_stage.at[p % NSLOT, 4])]

        cp_xd = pltpu.make_async_copy(x_hbm.at[:, pl.ds(0, RD), :], xd_raw, sem_in.at[0])
        cp_mem = pltpu.make_async_copy(mem_hbm, mem_v, sem_in.at[1])
        cp_wg = pltpu.make_async_copy(wg_hbm, wg_v, sem_in.at[2])
        cp_wu = pltpu.make_async_copy(wu_hbm, wu_v, sem_in.at[3])
        cp_wd = pltpu.make_async_copy(wd_hbm, wd_v, sem_in.at[4])

        cp_mem.start()
        cp_xd.start()
        cp_mem.wait()
        for cp in qkv_copies(0) + qkv_copies(1) + ox_copies(0):
            cp.start()

        def project(p, w0, w1):
            col = p * PW if isinstance(p, int) else pl.multiple_of(p * PW, 128)
            w = stage[p % NSLOT, w0 * PW:w1 * PW, :]
            sb = NSEG // PRB
            for b in range(PRB):
                y = jax.lax.dot_general(xd_v[b * sb * RD:(b + 1) * sb * RD, :], w, _NT,
                                        preferred_element_type=F32)
                y3 = y.reshape(sb, RD, (w1 - w0) * PW).astype(BF16)
                for which in range(w0, w1):
                    dst = (qd, kd, vd)[which]
                    dst[b * sb:(b + 1) * sb, :, pl.ds(col, PW)] = (
                        y3[:, :, (which - w0) * PW:(which - w0 + 1) * PW])
            wqkv[p, :, w0 * PW:w1 * PW] = pltpu.bitcast(w.T, jnp.uint32)

        def finish_ox(p):
            wo_v[p] = pltpu.bitcast(stage[p % NSLOT, 3 * PW:4 * PW, :], jnp.uint32)
            seg0 = p * SPP if isinstance(p, int) else pl.multiple_of(p * SPP, SPP)
            h_v[pl.ds(seg0, SPP), RD:SEG, :] = _ln(x_v[pl.ds(seg0, SPP), RD:SEG, :].astype(F32))

        cp_xd.wait()
        xd = xd_raw[...].astype(F32).reshape(ND, D)
        xd_v[...] = _ln(xd).astype(BF16)
        w_copy(0, 0).wait()
        for cp in qkv_copies(2) + ox_copies(1):
            cp.start()
        project(0, 0, 1)
        w_copy(0, 1).wait()
        w_copy(0, 2).wait()
        project(0, 1, 3)

        def pro_body(p, carry):
            for cp in qkv_copies(p) + ox_copies(p - 1):
                cp.wait()

            @pl.when(p + 2 < NP)
            def _():
                for cp in qkv_copies(p + 2):
                    cp.start()

            @pl.when(p + 1 < NP)
            def _():
                for cp in ox_copies(p + 1):
                    cp.start()

            project(p, 0, 3)
            finish_ox(p - 1)
            return carry

        jax.lax.fori_loop(1, NP, pro_body, 0)
        for cp in ox_copies(NP - 1):
            cp.wait()
        cp_wg.start()
        cp_wu.start()
        cp_wd.start()
        finish_ox(NP - 1)

        NK = 2 * (R1 + RD)
        row = jax.lax.broadcasted_iota(jnp.int32, (R1, NK), 0)
        lane = jax.lax.broadcasted_iota(jnp.int32, (R1, NK), 1)
        c_own_a = (lane < R1) | ((lane >= 2 * R1) & (lane < 2 * R1 + RD))
        c_own_b = jnp.logical_not(c_own_a)
        c_vis = (row < M) | (lane >= 2 * R1) | ((lane & (R1 - 1)) <= row)
        NKD = 2 * 2 * (M + RD)
        rowd = jax.lax.broadcasted_iota(jnp.int32, (2 * RD, NKD), 0)
        laned = jax.lax.broadcasted_iota(jnp.int32, (2 * RD, NKD), 1)
        same_seg = (rowd >= RD) == (laned >= NKD // 2)
        d_is_a = (laned & RD) == 0
        d_own_a = same_seg & d_is_a
        d_own_b = same_seg & jnp.logical_not(d_is_a)
        d_vis = ((laned & (2 * M)) == 0) | ((laned & (RD - 1)) <= (rowd & (RD - 1)))
        lane2 = jax.lax.broadcasted_iota(jnp.int32, (1, PW), 1)
        is_a2 = lane2 < DH

        def split_heads(d_ref, s, c0, c1):
            d = d_ref[s, :, c0:c1]
            z = jnp.zeros_like(d)
            return jnp.concatenate([jnp.where(is_a2, d, z), jnp.where(is_a2, z, d)], axis=0)

        def seg_step(s, half, m, xn, extras, erows, sched):
            l1 = jnp.concatenate([m, xn], axis=0).astype(BF16)

            def blockdiag(t, d2_ref, m2_ref, c0, c1):
                ta = jnp.where(is_a2, t, 0.0)
                tb = jnp.where(is_a2, 0.0, t)
                m2_ref[half, :, c0:c1] = jnp.concatenate(
                    [ta[0:M], tb[0:M]], axis=0).astype(BF16)
                return jnp.concatenate(
                    [ta.astype(BF16), tb.astype(BF16), split_heads(d2_ref, s, c0, c1)], axis=0)

            def stage_a(p):
                c0, c1 = p * PW, (p + 1) * PW
                y = jnp.dot(l1, pltpu.bitcast(wqkv[p], BF16), preferred_element_type=F32)
                qf = y[:, 0:PW].astype(BF16)
                kbd = blockdiag(y[:, PW:2 * PW], kd, km2, c0, c1)
                vbd = blockdiag(y[:, 2 * PW:3 * PW], vd, vm2, c0, c1)
                return qf, kbd, vbd

            def stage_b(qf, kbd):
                sc = jax.lax.dot_general(qf, kbd, _NT, preferred_element_type=F32) * scale
                return _pair_softmax(sc, c_vis, c_own_a, c_own_b)

            def stage_d(p, pm, vbd):
                c0, c1 = p * PW, (p + 1) * PW
                o_v[0:R1, c0:c1] = jnp.dot(pm, vbd, preferred_element_type=F32).astype(BF16)

            def stage_e(p0, p1):
                c0, c1 = p0 * PW, p1 * PW
                wo = pltpu.bitcast(wo_v[p0:p1].reshape((p1 - p0) * PW // 2, D), BF16)
                return jnp.dot(o_v[0:erows, c0:c1], wo, preferred_element_type=F32)

            def run(key):
                for fn in extras.get(key, ()):
                    fn()

            e_chunks, d_tail = sched
            pos_b = {p: p + 1 for p in range(NP)}
            pos_d = {p: p + 2 for p in range(NP - 2)}
            pos_d[NP - 2], pos_d[NP - 1] = NP + d_tail[0], NP + d_tail[1]
            abuf = {}
            pbuf = {}
            acc = None
            for t in range(NP + len(e_chunks)):
                if t < NP:
                    abuf[t] = stage_a(t)
                else:
                    part = stage_e(*e_chunks[t - NP])
                    acc = part if acc is None else acc + part
                run(t)
                for p in range(NP):
                    if pos_b[p] == t:
                        pbuf[p] = stage_b(abuf[p][0], abuf[p][1])
                for p in range(NP):
                    if pos_d[p] == t:
                        stage_d(p, pbuf[p], abuf[p][2])
                run(("post", t))
            h_v[s, RD:SEG, :] = x_v[s, RD:SEG, :].astype(F32) + acc[M:R1]
            return acc

        def da_qk(s0, p):
            c0, c1 = p * PW, (p + 1) * PW
            q = jnp.concatenate([qd[s0, :, c0:c1], qd[s0 + 1, :, c0:c1]], axis=0)
            k = jnp.concatenate([km2[0, :, c0:c1], split_heads(kd, s0, c0, c1),
                                 km2[1, :, c0:c1], split_heads(kd, s0 + 1, c0, c1)], axis=0)
            sc = jax.lax.dot_general(q, k, _NT, preferred_element_type=F32) * scale
            return _pair_softmax(sc, d_vis, d_own_a, d_own_b)

        def da_pv(s0, p, pm):
            c0, c1 = p * PW, (p + 1) * PW
            v = jnp.concatenate([vm2[0, :, c0:c1], split_heads(vd, s0, c0, c1),
                                 vm2[1, :, c0:c1], split_heads(vd, s0 + 1, c0, c1)], axis=0)
            o_v[R1:R1 + 2 * RD, c0:c1] = jnp.dot(pm, v, preferred_element_type=F32).astype(BF16)

        def out_copy(s0, n, k):
            return pltpu.make_async_copy(
                out_v.at[pl.ds(s0, n)], out_hbm.at[pl.ds(s0, n)], sem_out.at[k])

        def main_body(j, m, first=False):
            s0 = 0 if first else pl.multiple_of(2 * j, 2)
            xn0 = h_v[s0, RD:SEG, :]
            xn1 = h_v[s0 + 1, RD:SEG, :]
            pieces = []
            if not first:
                s1 = pl.multiple_of((j - 1) * 2, 2)
                s2 = pl.multiple_of(jnp.maximum(j - 2, 0) * 2, 2)
                hb_v[...] = jnp.concatenate(
                    [h_v[s2, 0:RD, :], h_v[s2 + 1, 0:RD, :],
                     h_v[s1, RD:SEG, :], h_v[s1 + 1, RD:SEG, :]], axis=0)
                hn = _ln(hb_v[...]).astype(BF16)

                gbuf = {}

                def gate(c):
                    gbuf[c] = jnp.dot(hn, wg_v[:, c * FW:(c + 1) * FW], preferred_element_type=F32)

                def up(c):
                    u = jnp.dot(hn, wu_v[:, c * FW:(c + 1) * FW], preferred_element_type=F32)
                    g = gbuf[c]
                    act_v[:, c * FW:(c + 1) * FW] = (g * jax.nn.sigmoid(g) * u).astype(BF16)

                def down(n, half):
                    n0, n1 = n * 128, (n + 1) * 128
                    f0, f1 = half * (F // 2), (half + 1) * (F // 2)
                    y = hb_v[:, n0:n1] + jnp.dot(act_v[:, f0:f1], wd_v[f0:f1, n0:n1],
                                                 preferred_element_type=F32)
                    if half == 0:
                        hb_v[:, n0:n1] = y
                    else:
                        y = y.astype(BF16)
                        out_v[s2, 0:RD, n0:n1] = y[0:RD]
                        out_v[s2 + 1, 0:RD, n0:n1] = y[RD:2 * RD]
                        out_v[s1, RD:SEG, n0:n1] = y[2 * RD:2 * RD + RP]
                        out_v[s1 + 1, RD:SEG, n0:n1] = y[2 * RD + RP:FR]

                for c in range(FC):
                    pieces += [functools.partial(gate, c), functools.partial(up, c)]
                for half in range(2):
                    pieces += [functools.partial(down, n, half) for n in range(D // 128)]
            na = NP
            nb = len(pieces) - 2 * NP

            extras = {} if first else {t + 1: [pieces[t]] for t in range(na)}
            acc = seg_step(s0, 0, m, xn0, extras, R1, SCHED_A)
            for fn in pieces[na:na + nb]:
                fn()

            pd = {}

            def qk(p):
                pd[p] = da_qk(s0, p)

            def pv(p):
                da_pv(s0, p, pd[p])

            extras = {} if first else {t + 1: [pieces[na + nb + t]] for t in range(NP)}
            for p in range(NP):
                extras.setdefault(("post", NP + DA_QK_AT[p]), []).append(functools.partial(qk, p))
                extras.setdefault(("post", NP + DA_PV_AT[p]), []).append(functools.partial(pv, p))
            acc = seg_step(s0 + 1, 1, acc[0:M], xn1, extras, R1 if first else R1 + 2 * RD,
                           SCHED_B0 if first else SCHED_B)
            if not first:
                h_v[s1, 0:RD, :] = x_v[s1, 0:RD, :].astype(F32) + acc[R1:R1 + RD]
                h_v[s1 + 1, 0:RD, :] = x_v[s1 + 1, 0:RD, :].astype(F32) + acc[R1 + RD:R1 + 2 * RD]

                @pl.when(j >= 2)
                def _():
                    out_copy(s2, 2, j - 2).start()
            return acc[0:M]

        h_v[0:2, 0:RD, :] = jnp.zeros((2, RD, D), F32)
        m1 = main_body(0, mem_v[...].astype(F32), first=True)
        cp_wg.wait()
        cp_wu.wait()
        cp_wd.wait()
        jax.lax.fori_loop(1, NJ, main_body, m1)

        sl = NSEG - 2
        a = jnp.dot(o_v[R1:R1 + 2 * RD, :], pltpu.bitcast(wo_v[...].reshape(H * DH // 2, D), BF16),
                    preferred_element_type=F32)
        hl0 = x_v[sl, 0:RD, :].astype(F32) + a[0:RD]
        hl1 = x_v[sl + 1, 0:RD, :].astype(F32) + a[RD:2 * RD]
        h = jnp.concatenate([h_v[sl - 2, 0:RD, :], h_v[sl - 1, 0:RD, :],
                             hl0, h_v[sl, RD:SEG, :], hl1, h_v[sl + 1, RD:SEG, :]], axis=0)
        hn = _ln(h).astype(BF16)
        g = jnp.dot(hn, wg_v[...], preferred_element_type=F32)
        u = jnp.dot(hn, wu_v[...], preferred_element_type=F32)
        act = (g * jax.nn.sigmoid(g) * u).astype(BF16)
        y = (h + jnp.dot(act, wd_v[...], preferred_element_type=F32)).astype(BF16)
        out_v[sl - 2, 0:RD, :] = y[0:RD]
        out_v[sl - 1, 0:RD, :] = y[RD:2 * RD]
        out_v[sl] = y[2 * RD:2 * RD + SEG]
        out_v[sl + 1] = y[2 * RD + SEG:2 * RD + 2 * SEG]
        out_copy(sl - 2, 4, NJ - 2).start()

        for j in range(2, NJ):
            out_copy(2 * j - 4, 2, j - 2).wait()
        out_copy(sl - 2, 4, NJ - 2).wait()

    scratch = [
        pltpu.VMEM((NSEG, SEG, D), BF16),
        pltpu.VMEM((M, D), BF16),
        pltpu.VMEM((NSLOT, 4 * PW, D), BF16),
        pltpu.VMEM((NP, D // 2, 3 * PW), jnp.uint32),
        pltpu.VMEM((NP, PW // 2, D), jnp.uint32),
        pltpu.VMEM((D, F), BF16),
        pltpu.VMEM((D, F), BF16),
        pltpu.VMEM((F, D), BF16),
        pltpu.VMEM((NSEG, RD, D), BF16),
        pltpu.VMEM((ND, D), BF16),
        pltpu.VMEM((NSEG, RD, H * DH), BF16),
        pltpu.VMEM((NSEG, RD, H * DH), BF16),
        pltpu.VMEM((NSEG, RD, H * DH), BF16),
        pltpu.VMEM((2, 2 * M, H * DH), BF16),
        pltpu.VMEM((2, 2 * M, H * DH), BF16),
        pltpu.VMEM((NSEG, SEG, D), F32),
        pltpu.VMEM((NSEG, SEG, D), BF16),
        pltpu.VMEM((R1 + 2 * RD, H * DH), BF16),
        pltpu.VMEM((FR, D), F32),
        pltpu.VMEM((FR, F), BF16),
        pltpu.SemaphoreType.DMA((5,)),
        pltpu.SemaphoreType.DMA((NSLOT, 5)),
        pltpu.SemaphoreType.DMA((NJ,)),
    ]
    return kernel, scratch


@functools.partial(jax.jit, static_argnames=("seg",))
def _impl(A_x, A_mem0, A_Wq, A_Wk, A_Wv, A_Wo, B_w_gate, B_w_up, B_w_down, *, seg):
    B, S, D = A_x.shape
    _, H, DH = A_Wq.shape
    M = A_mem0.shape[1]
    F = B_w_gate.shape[1]
    assert B == 1 and S % seg == 0 and seg == 32 and M == 8
    nseg = S // seg

    kernel, scratch = _make_kernel(S, D, H, DH, M, seg, F)

    x3 = A_x.reshape(nseg, seg, D)
    mem = A_mem0.reshape(M, D)
    wqT = jnp.transpose(A_Wq, (1, 2, 0)).reshape(H * DH, D)
    wkT = jnp.transpose(A_Wk, (1, 2, 0)).reshape(H * DH, D)
    wvT = jnp.transpose(A_Wv, (1, 2, 0)).reshape(H * DH, D)
    wo = A_Wo.reshape(H * DH, D)

    out = pl.pallas_call(
        kernel,
        out_shape=jax.ShapeDtypeStruct((nseg, seg, D), A_x.dtype),
        in_specs=[pl.BlockSpec(memory_space=pl.ANY)] * 9,
        out_specs=pl.BlockSpec(memory_space=pl.ANY),
        scratch_shapes=scratch,
        compiler_params=pltpu.CompilerParams(vmem_limit_bytes=110 * 1024 * 1024, disable_bounds_checks=True, disable_semaphore_checks=True),
    )(x3, mem, wqT, wkT, wvT, wo, B_w_gate, B_w_up, B_w_down)
    return out.reshape(B, S, D)


def pallas_sequential_preLN__memory_aug_recurrent_mem_tr__swiglu_ffn__prompt_kernel(
    A_x,
    A_mem0,
    A_Wq,
    A_Wk,
    A_Wv,
    A_Wo,
    A_seg_len,
    B_x,
    B_w_gate,
    B_w_up,
    B_w_down,
):
    seg = A_seg_len if isinstance(A_seg_len, int) else 32
    return _impl(A_x, A_mem0, A_Wq, A_Wk, A_Wv, A_Wo, B_w_gate, B_w_up, B_w_down, seg=seg)
```

```python
import functools

import jax
import jax.numpy as jnp
import jax.experimental.pallas as pl
import jax.experimental.pallas.tpu as pltpu

F32 = jnp.float32
BF16 = jnp.bfloat16

_NT = (((1,), (1,)), ((), ()))
_NEG = -1000000000.0


def _ln(x):
    m = jnp.mean(x, axis=-1, keepdims=True)
    xc = x - m
    v = jnp.mean(xc * xc, axis=-1, keepdims=True)
    return xc * jax.lax.rsqrt(v + 1e-05)


def _pair_softmax(sc, visible, own_a, own_b):
    sc = jnp.where(visible, sc, _NEG)
    sa_ = jnp.where(own_a, sc, -jnp.inf)
    sb_ = jnp.where(own_b, sc, -jnp.inf)
    ma = jnp.max(sa_, axis=1, keepdims=True)
    mb = jnp.max(sb_, axis=1, keepdims=True)
    e = jnp.exp(jnp.where(own_a, sa_ - ma, sb_ - mb))
    da = jnp.sum(jnp.where(own_a, e, 0.0), axis=1, keepdims=True)
    db = jnp.sum(jnp.where(own_a, 0.0, e), axis=1, keepdims=True)
    return (e / jnp.where(own_a, da, db)).astype(BF16)


def _make_kernel(S, D, H, DH, M, SEG, F):
    NSEG = S // SEG
    NP = H // 2
    PW = 2 * DH
    RD = M
    RP = SEG - RD
    R1 = M + RP
    ND = NSEG * RD
    NSLOT = 3
    PRB = 4
    SPP = NSEG // NP
    NJ = NSEG // 2
    FW = 128
    FC = F // FW
    FR = 2 * SEG
    SCHED_A = (((0, 2), (2, 5), (5, 8), (8, 16)), (0, 1, 2))
    SCHED_B = (tuple((p, p + 1) for p in range(NP)), (1, 2, 4))
    SCHED_B0 = (tuple((p, p + 1) for p in range(NP)), (1, 4, 5))
    ORDER = 'xdb'
    ORDER0 = 'xbd'
    LAGD = 3
    DSPLIT = 2
    SLOTS_A = tuple(range(1, 17))
    SLOTS_B = tuple(range(1, 17))
    QKF = 0.8
    DA_QK_AT = tuple(0 + int(p * QKF) for p in range(NP))
    DA_PV_AT = tuple(min(NP - 1, max(p, DA_QK_AT[p] + 3)) for p in range(NP))
    assert all(0 <= a < b < NP for a, b in zip(DA_QK_AT, DA_PV_AT))
    scale = float(DH) ** -0.5
    LAG_B = 1
    LAG_D = 2
    E_CHUNKS = ((0, 3), (3, 6), (6, 9), (9, 12), (12, 16))

    def kernel(x_hbm, mem_hbm, wq_hbm, wk_hbm, wv_hbm, wo_hbm, wg_hbm, wu_hbm, wd_hbm,
               out_hbm,
               x_v, mem_v, stage, wqkv, wo_v, wg_v, wu_v, wd_v,
               xd_raw, xd_v, qd, kd2, vd2, km2, vm2, h_v, out_v, o_v, hb_v, act_v,
               sem_in, sem_stage, sem_out):
        w_hbm = (wq_hbm, wk_hbm, wv_hbm, wo_hbm)

        def w_copy(p, which):
            slot = p % NSLOT
            return pltpu.make_async_copy(
                w_hbm[which].at[pl.ds(p * PW, PW), :],
                stage.at[slot, pl.ds(which * PW, PW), :], sem_stage.at[slot, which])

        def qkv_copies(p):
            return [w_copy(p, which) for which in range(3)]

        def ox_copies(p):
            return [w_copy(p, 3), pltpu.make_async_copy(
                x_hbm.at[pl.ds(p * SPP, SPP)], x_v.at[pl.ds(p * SPP, SPP)],
                sem_stage.at[p % NSLOT, 4])]

        cp_xd = pltpu.make_async_copy(x_hbm.at[:, pl.ds(0, RD), :], xd_raw, sem_in.at[0])
        cp_mem = pltpu.make_async_copy(mem_hbm, mem_v, sem_in.at[1])
        cp_wg = pltpu.make_async_copy(wg_hbm, wg_v, sem_in.at[2])
        cp_wu = pltpu.make_async_copy(wu_hbm, wu_v, sem_in.at[3])
        cp_wd = pltpu.make_async_copy(wd_hbm, wd_v, sem_in.at[4])

        cp_mem.start()
        cp_xd.start()
        cp_mem.wait()
        for cp in qkv_copies(0) + qkv_copies(1) + ox_copies(0):
            cp.start()

        lane_p = jax.lax.broadcasted_iota(jnp.int32, (1, 1, PW), 2)
        is_a3 = lane_p < DH

        def project(p, w0, w1):
            col = p * PW if isinstance(p, int) else pl.multiple_of(p * PW, 128)
            w = stage[p % NSLOT, w0 * PW:w1 * PW, :]
            sb = NSEG // PRB
            for b in range(PRB):
                y = jax.lax.dot_general(xd_v[b * sb * RD:(b + 1) * sb * RD, :], w, _NT,
                                        preferred_element_type=F32)
                y3 = y.reshape(sb, RD, (w1 - w0) * PW)
                for which in range(w0, w1):
                    yw = y3[:, :, (which - w0) * PW:(which - w0 + 1) * PW]
                    if which == 0:
                        qd[b * sb:(b + 1) * sb, :, pl.ds(col, PW)] = yw.astype(BF16)
                    else:
                        ya = jnp.where(is_a3, yw, 0.0)
                        yb = jnp.where(is_a3, 0.0, yw)
                        dst = kd2 if which == 1 else vd2
                        dst[b * sb:(b + 1) * sb, :, pl.ds(col, PW)] = pltpu.bitcast(
                            jnp.concatenate([ya, yb], axis=1).astype(BF16), jnp.uint32)
            wqkv[p, :, w0 * PW:w1 * PW] = pltpu.bitcast(w.T, jnp.uint32)

        def finish_ox(p):
            wo_v[p] = pltpu.bitcast(stage[p % NSLOT, 3 * PW:4 * PW, :], jnp.uint32)
            seg0 = p * SPP if isinstance(p, int) else pl.multiple_of(p * SPP, SPP)
            h_v[pl.ds(seg0, SPP), RD:SEG, :] = _ln(x_v[pl.ds(seg0, SPP), RD:SEG, :].astype(F32))

        cp_xd.wait()
        xd = xd_raw[...].astype(F32).reshape(ND, D)
        xd_v[...] = _ln(xd).astype(BF16)
        w_copy(0, 0).wait()
        for cp in qkv_copies(2) + ox_copies(1):
            cp.start()
        project(0, 0, 1)
        w_copy(0, 1).wait()
        w_copy(0, 2).wait()
        project(0, 1, 3)

        def pro_body(p, carry):
            for cp in qkv_copies(p) + ox_copies(p - 1):
                cp.wait()

            @pl.when(p + 2 < NP)
            def _():
                for cp in qkv_copies(p + 2):
                    cp.start()

            @pl.when(p + 1 < NP)
            def _():
                for cp in ox_copies(p + 1):
                    cp.start()

            project(p, 0, 3)
            finish_ox(p - 1)
            return carry

        jax.lax.fori_loop(1, NP, pro_body, 0)
        for cp in ox_copies(NP - 1):
            cp.wait()
        cp_wg.start()
        cp_wu.start()
        cp_wd.start()
        finish_ox(NP - 1)

        NK = 2 * (R1 + RD)
        row = jax.lax.broadcasted_iota(jnp.int32, (R1, NK), 0)
        lane = jax.lax.broadcasted_iota(jnp.int32, (R1, NK), 1)
        c_own_a = (lane < R1) | ((lane >= 2 * R1) & (lane < 2 * R1 + RD))
        c_own_b = jnp.logical_not(c_own_a)
        c_vis = (row < M) | (lane >= 2 * R1) | ((lane & (R1 - 1)) <= row)
        NKD = 2 * 2 * (M + RD)
        rowd = jax.lax.broadcasted_iota(jnp.int32, (2 * RD, NKD), 0)
        laned = jax.lax.broadcasted_iota(jnp.int32, (2 * RD, NKD), 1)
        same_seg = (rowd >= RD) == (laned >= NKD // 2)
        d_is_a = (laned & RD) == 0
        d_own_a = same_seg & d_is_a
        d_own_b = same_seg & jnp.logical_not(d_is_a)
        d_vis = ((laned & (2 * M)) == 0) | ((laned & (RD - 1)) <= (rowd & (RD - 1)))
        lane2 = jax.lax.broadcasted_iota(jnp.int32, (1, PW), 1)
        is_a2 = lane2 < DH

        def seg_step(s, half, m, xn, extras, erows, sched, order):
            l1 = jnp.concatenate([m, xn], axis=0).astype(BF16)

            def blockdiag(t, d2_ref, m2_ref, c0, c1):
                ta = jnp.where(is_a2, t, 0.0)
                tb = jnp.where(is_a2, 0.0, t)
                m2_ref[half, :, c0:c1] = pltpu.bitcast(jnp.concatenate(
                    [ta[0:M], tb[0:M]], axis=0).astype(BF16), jnp.uint32)
                return jnp.concatenate(
                    [ta.astype(BF16), tb.astype(BF16), pltpu.bitcast(d2_ref[s, :, c0:c1], BF16)], axis=0)

            def stage_a(p):
                c0, c1 = p * PW, (p + 1) * PW
                y = jnp.dot(l1, pltpu.bitcast(wqkv[p], BF16), preferred_element_type=F32)
                qf = y[:, 0:PW].astype(BF16)
                kbd = blockdiag(y[:, PW:2 * PW], kd2, km2, c0, c1)
                vbd = blockdiag(y[:, 2 * PW:3 * PW], vd2, vm2, c0, c1)
                return qf, kbd, vbd

            def stage_b(qf, kbd):
                sc = jax.lax.dot_general(qf, kbd, _NT, preferred_element_type=F32) * scale
                return _pair_softmax(sc, c_vis, c_own_a, c_own_b)

            def stage_d(p, pm, vbd):
                c0, c1 = p * PW, (p + 1) * PW
                o_v[0:R1 // 2, c0:c1] = pltpu.bitcast(
                    jnp.dot(pm, vbd, preferred_element_type=F32).astype(BF16), jnp.uint32)

            def stage_e(p0, p1):
                c0, c1 = p0 * PW, p1 * PW
                wo = pltpu.bitcast(wo_v[p0:p1].reshape((p1 - p0) * PW // 2, D), BF16)
                return jnp.dot(pltpu.bitcast(o_v[0:erows // 2, c0:c1], BF16), wo,
                               preferred_element_type=F32)

            ran = set()

            def run(key):
                if key in extras:
                    ran.add(key)
                for fn in extras.get(key, ()):
                    fn()

            e_chunks, d_tail = sched
            pos_b = {p: p + 1 for p in range(NP)}
            pos_d = {p: p + LAGD for p in range(NP - len(d_tail))}
            for i, dt in enumerate(d_tail):
                pos_d[NP - len(d_tail) + i] = NP + dt
            abuf = {}
            pbuf = {}
            acc = None
            for t in range(NP + len(e_chunks)):
                if t < NP:
                    abuf[t] = stage_a(t)
                else:
                    part = stage_e(*e_chunks[t - NP])
                    acc = part if acc is None else acc + part
                def do_b():
                    for p in range(NP):
                        if pos_b[p] == t:
                            pbuf[p] = stage_b(abuf[p][0], abuf[p][1])

                def do_d():
                    for p in range(NP):
                        if pos_d[p] == t:
                            stage_d(p, pbuf[p], abuf[p][2])

                for ch in order:
                    if ch == "x":
                        run(t)
                    elif ch == "b":
                        do_b()
                    else:
                        do_d()
                run(("post", t))
            assert ran == set(extras), (ran, set(extras))
            h_v[s, RD:SEG, :] = x_v[s, RD:SEG, :].astype(F32) + acc[M:R1]
            return acc

        def da_qk(s0, p):
            c0, c1 = p * PW, (p + 1) * PW
            q = jnp.concatenate([qd[s0, :, c0:c1], qd[s0 + 1, :, c0:c1]], axis=0)
            k = pltpu.bitcast(jnp.concatenate(
                [km2[0, :, c0:c1], kd2[s0, :, c0:c1],
                 km2[1, :, c0:c1], kd2[s0 + 1, :, c0:c1]], axis=0), BF16)
            sc = jax.lax.dot_general(q, k, _NT, preferred_element_type=F32) * scale
            return _pair_softmax(sc, d_vis, d_own_a, d_own_b)

        def da_pv(s0, p, pm):
            c0, c1 = p * PW, (p + 1) * PW
            v = pltpu.bitcast(jnp.concatenate(
                [vm2[0, :, c0:c1], vd2[s0, :, c0:c1],
                 vm2[1, :, c0:c1], vd2[s0 + 1, :, c0:c1]], axis=0), BF16)
            o_v[R1 // 2:R1 // 2 + RD, c0:c1] = pltpu.bitcast(
                jnp.dot(pm, v, preferred_element_type=F32).astype(BF16), jnp.uint32)

        def out_copy(s0, n, k):
            return pltpu.make_async_copy(
                out_v.at[pl.ds(s0, n)], out_hbm.at[pl.ds(s0, n)], sem_out.at[k])

        def main_body(j, m, first=False):
            s0 = 0 if first else pl.multiple_of(2 * j, 2)
            xn0 = h_v[s0, RD:SEG, :]
            xn1 = h_v[s0 + 1, RD:SEG, :]
            pieces = []
            if not first:
                s1 = pl.multiple_of((j - 1) * 2, 2)
                s2 = pl.multiple_of(jnp.maximum(j - 2, 0) * 2, 2)
                hb_v[...] = jnp.concatenate(
                    [h_v[s2, 0:RD, :], h_v[s2 + 1, 0:RD, :],
                     h_v[s1, RD:SEG, :], h_v[s1 + 1, RD:SEG, :]], axis=0)
                hn = _ln(hb_v[...]).astype(BF16)

                gbuf = {}

                def gate(c):
                    gbuf[c] = jnp.dot(hn, wg_v[:, c * FW:(c + 1) * FW], preferred_element_type=F32)

                def up(c):
                    u = jnp.dot(hn, wu_v[:, c * FW:(c + 1) * FW], preferred_element_type=F32)
                    g = gbuf[c]
                    act_v[:, c * FW:(c + 1) * FW] = pltpu.bitcast(
                        (g * jax.nn.sigmoid(g) * u).astype(BF16), jnp.uint32)

                def down(n, part):
                    n0, n1 = n * 128, (n + 1) * 128
                    f0, f1 = part * (F // DSPLIT), (part + 1) * (F // DSPLIT)
                    y = hb_v[:, n0:n1] + jnp.dot(pltpu.bitcast(act_v[:, f0:f1], BF16), wd_v[f0:f1, n0:n1],
                                                 preferred_element_type=F32)
                    if part < DSPLIT - 1:
                        hb_v[:, n0:n1] = y
                    else:
                        y = y.astype(BF16)
                        out_v[s2, 0:RD, n0:n1] = y[0:RD]
                        out_v[s2 + 1, 0:RD, n0:n1] = y[RD:2 * RD]
                        out_v[s1, RD:SEG, n0:n1] = y[2 * RD:2 * RD + RP]
                        out_v[s1 + 1, RD:SEG, n0:n1] = y[2 * RD + RP:FR]

                for c in range(FC):
                    pieces += [functools.partial(gate, c), functools.partial(up, c)]
                for part in range(DSPLIT):
                    pieces += [functools.partial(down, n, part) for n in range(D // 128)]
            na = len(SLOTS_A)
            nb = len(pieces) - len(SLOTS_A) - len(SLOTS_B)

            extras = {}
            if not first:
                for i, t in enumerate(SLOTS_A):
                    extras.setdefault(t, []).append(pieces[i])
            acc = seg_step(s0, 0, m, xn0, extras, R1, SCHED_A, ORDER0 if first else ORDER)
            for fn in pieces[na:na + nb]:
                fn()

            pd = {}

            def qk(p):
                pd[p] = da_qk(s0, p)

            def pv(p):
                da_pv(s0, p, pd[p])

            extras = {}
            if not first:
                for i, t in enumerate(SLOTS_B):
                    extras.setdefault(t, []).append(pieces[na + nb + i])
            for p in range(NP):
                extras.setdefault(("post", NP + DA_QK_AT[p]), []).append(functools.partial(qk, p))
                extras.setdefault(("post", NP + DA_PV_AT[p]), []).append(functools.partial(pv, p))
            acc = seg_step(s0 + 1, 1, acc[0:M], xn1, extras, R1 if first else R1 + 2 * RD,
                           SCHED_B0 if first else SCHED_B, ORDER0 if first else ORDER)
            if not first:
                h_v[s1, 0:RD, :] = x_v[s1, 0:RD, :].astype(F32) + acc[R1:R1 + RD]
                h_v[s1 + 1, 0:RD, :] = x_v[s1 + 1, 0:RD, :].astype(F32) + acc[R1 + RD:R1 + 2 * RD]

                @pl.when(j >= 2)
                def _():
                    out_copy(s2, 2, j - 2).start()
            return acc[0:M]

        h_v[0:2, 0:RD, :] = jnp.zeros((2, RD, D), F32)
        m1 = main_body(0, mem_v[...].astype(F32), first=True)
        cp_wg.wait()
        cp_wu.wait()
        cp_wd.wait()
        jax.lax.fori_loop(1, NJ, main_body, m1)

        sl = NSEG - 2
        a = jnp.dot(pltpu.bitcast(o_v[R1 // 2:R1 // 2 + RD, :], BF16), pltpu.bitcast(wo_v[...].reshape(H * DH // 2, D), BF16),
                    preferred_element_type=F32)
        hl0 = x_v[sl, 0:RD, :].astype(F32) + a[0:RD]
        hl1 = x_v[sl + 1, 0:RD, :].astype(F32) + a[RD:2 * RD]
        h = jnp.concatenate([h_v[sl - 2, 0:RD, :], h_v[sl - 1, 0:RD, :],
                             hl0, h_v[sl, RD:SEG, :], hl1, h_v[sl + 1, RD:SEG, :]], axis=0)
        hn = _ln(h).astype(BF16)
        g = jnp.dot(hn, wg_v[...], preferred_element_type=F32)
        u = jnp.dot(hn, wu_v[...], preferred_element_type=F32)
        act = (g * jax.nn.sigmoid(g) * u).astype(BF16)
        y = (h + jnp.dot(act, wd_v[...], preferred_element_type=F32)).astype(BF16)
        out_v[sl - 2, 0:RD, :] = y[0:RD]
        out_v[sl - 1, 0:RD, :] = y[RD:2 * RD]
        out_v[sl] = y[2 * RD:2 * RD + SEG]
        out_v[sl + 1] = y[2 * RD + SEG:2 * RD + 2 * SEG]
        out_copy(sl - 2, 4, NJ - 2).start()

        for j in range(2, NJ):
            out_copy(2 * j - 4, 2, j - 2).wait()
        out_copy(sl - 2, 4, NJ - 2).wait()

    scratch = [
        pltpu.VMEM((NSEG, SEG, D), BF16),
        pltpu.VMEM((M, D), BF16),
        pltpu.VMEM((NSLOT, 4 * PW, D), BF16),
        pltpu.VMEM((NP, D // 2, 3 * PW), jnp.uint32),
        pltpu.VMEM((NP, PW // 2, D), jnp.uint32),
        pltpu.VMEM((D, F), BF16),
        pltpu.VMEM((D, F), BF16),
        pltpu.VMEM((F, D), BF16),
        pltpu.VMEM((NSEG, RD, D), BF16),
        pltpu.VMEM((ND, D), BF16),
        pltpu.VMEM((NSEG, RD, H * DH), BF16),
        pltpu.VMEM((NSEG, RD, H * DH), jnp.uint32),
        pltpu.VMEM((NSEG, RD, H * DH), jnp.uint32),
        pltpu.VMEM((2, M, H * DH), jnp.uint32),
        pltpu.VMEM((2, M, H * DH), jnp.uint32),
        pltpu.VMEM((NSEG, SEG, D), F32),
        pltpu.VMEM((NSEG, SEG, D), BF16),
        pltpu.VMEM((R1 // 2 + RD, H * DH), jnp.uint32),
        pltpu.VMEM((FR, D), F32),
        pltpu.VMEM((FR // 2, F), jnp.uint32),
        pltpu.SemaphoreType.DMA((5,)),
        pltpu.SemaphoreType.DMA((NSLOT, 5)),
        pltpu.SemaphoreType.DMA((NJ,)),
    ]
    return kernel, scratch


@functools.partial(jax.jit, static_argnames=("seg",))
def _impl(A_x, A_mem0, A_Wq, A_Wk, A_Wv, A_Wo, B_w_gate, B_w_up, B_w_down, *, seg):
    B, S, D = A_x.shape
    _, H, DH = A_Wq.shape
    M = A_mem0.shape[1]
    F = B_w_gate.shape[1]
    assert B == 1 and S % seg == 0 and seg == 32 and M == 8
    nseg = S // seg

    kernel, scratch = _make_kernel(S, D, H, DH, M, seg, F)

    x3 = A_x.reshape(nseg, seg, D)
    mem = A_mem0.reshape(M, D)
    wqT = jnp.transpose(A_Wq, (1, 2, 0)).reshape(H * DH, D)
    wkT = jnp.transpose(A_Wk, (1, 2, 0)).reshape(H * DH, D)
    wvT = jnp.transpose(A_Wv, (1, 2, 0)).reshape(H * DH, D)
    wo = A_Wo.reshape(H * DH, D)

    out = pl.pallas_call(
        kernel,
        out_shape=jax.ShapeDtypeStruct((nseg, seg, D), A_x.dtype),
        in_specs=[pl.BlockSpec(memory_space=pl.ANY)] * 9,
        out_specs=pl.BlockSpec(memory_space=pl.ANY),
        scratch_shapes=scratch,
        compiler_params=pltpu.CompilerParams(vmem_limit_bytes=110 * 1024 * 1024, disable_bounds_checks=True, disable_semaphore_checks=True),
    )(x3, mem, wqT, wkT, wvT, wo, B_w_gate, B_w_up, B_w_down)
    return out.reshape(B, S, D)


def pallas_sequential_preLN__memory_aug_recurrent_mem_tr__swiglu_ffn__prompt_kernel(
    A_x,
    A_mem0,
    A_Wq,
    A_Wk,
    A_Wv,
    A_Wo,
    A_seg_len,
    B_x,
    B_w_gate,
    B_w_up,
    B_w_down,
):
    seg = A_seg_len if isinstance(A_seg_len, int) else 32
    return _impl(A_x, A_mem0, A_Wq, A_Wk, A_Wv, A_Wo, B_w_gate, B_w_up, B_w_down, seg=seg)
```

```python
import functools

import jax
import jax.numpy as jnp
import jax.experimental.pallas as pl
import jax.experimental.pallas.tpu as pltpu

F32 = jnp.float32
BF16 = jnp.bfloat16

_NT = (((1,), (1,)), ((), ()))
_NEG = -1000000000.0


def _ln(x):
    m = jnp.mean(x, axis=-1, keepdims=True)
    xc = x - m
    v = jnp.mean(xc * xc, axis=-1, keepdims=True)
    return xc * jax.lax.rsqrt(v + 1e-05)


def _pair_softmax(sc, visible, own_a, own_b):
    sc = jnp.where(visible, sc, _NEG)
    sa_ = jnp.where(own_a, sc, -jnp.inf)
    sb_ = jnp.where(own_b, sc, -jnp.inf)
    ma = jnp.max(sa_, axis=1, keepdims=True)
    mb = jnp.max(sb_, axis=1, keepdims=True)
    e = jnp.exp(jnp.where(own_a, sa_ - ma, sb_ - mb))
    da = jnp.sum(jnp.where(own_a, e, 0.0), axis=1, keepdims=True)
    db = jnp.sum(jnp.where(own_a, 0.0, e), axis=1, keepdims=True)
    return (e / jnp.where(own_a, da, db)).astype(BF16)


def _make_kernel(S, D, H, DH, M, SEG, F):
    NSEG = S // SEG
    NP = H // 2
    PW = 2 * DH
    RD = M
    RP = SEG - RD
    R1 = M + RP
    ND = NSEG * RD
    NSLOT = 3
    PRB = 4
    SPP = NSEG // NP
    NJ = NSEG // 2
    FW = 128
    FC = F // FW
    FR = 2 * SEG
    DSPLIT = 2
    LAGW = 4
    LAGE = 6
    FB_STEPS = (1, 2, 3, 4, 5, 7, 9, 11)
    AE_ORDER = (1, 0, 2)
    ESPLIT = 1

    def steps(second):
        prog = []
        for t in range(NP):
            if second and t >= LAGE and ESPLIT:
                prog.append(("AE", t, t - LAGE))
            else:
                prog.append(("A", t))
                if second and t >= LAGE:
                    prog.append(("E", t - LAGE, t - LAGE + 1))
            if t >= 1 and (not second or t in FB_STEPS):
                prog.append(("F",))
            if t >= 3:
                prog.append(("D", t - 3))
            if second and t >= LAGW:
                prog.append(("W", t - LAGW))
            if t >= 1:
                prog += [("B", t - 1), ("V", t - 1)]
        prog.append(("V", NP - 1))
        return prog

    F_ = ("F",)
    PROG_A = steps(False) + [("E", 0, 2), F_, ("D", 13), ("B", 15), ("E", 2, 5), ("D", 14), ("E", 5, 8), ("D", 15), ("E", 8, 16), F_, F_]
    PROG_B = steps(True) + [("E", 10, 11), ("W", 12), F_, ("D", 13), ("B", 15), ("E", 11, 12), ("W", 13), F_, F_, ("E", 12, 13), ("D", 14), ("W", 14), F_, F_, ("E", 13, 14), ("D", 15), ("W", 15), F_, F_, F_, ("E", 14, 16)]
    scale = float(DH) ** -0.5

    def kernel(x_hbm, mem_hbm, wq_hbm, wk_hbm, wv_hbm, wo_hbm, wg_hbm, wu_hbm, wd_hbm,
               out_hbm,
               x_v, mem_v, stage, wqkv, wo_v, wg_v, wu_v, wd_v,
               xd_raw, xd_v, qd, kd2, vd2, kf, vm2, h_v, out_v, o_v, hb_v, act_v,
               sem_in, sem_stage, sem_out):
        w_hbm = (wq_hbm, wk_hbm, wv_hbm, wo_hbm)

        def w_copy(p, which):
            slot = p % NSLOT
            return pltpu.make_async_copy(
                w_hbm[which].at[pl.ds(p * PW, PW), :],
                stage.at[slot, pl.ds(which * PW, PW), :], sem_stage.at[slot, which])

        def qkv_copies(p):
            return [w_copy(p, which) for which in range(3)]

        def ox_copies(p):
            return [w_copy(p, 3), pltpu.make_async_copy(
                x_hbm.at[pl.ds(p * SPP, SPP)], x_v.at[pl.ds(p * SPP, SPP)],
                sem_stage.at[p % NSLOT, 4])]

        cp_xd = pltpu.make_async_copy(x_hbm.at[:, pl.ds(0, RD), :], xd_raw, sem_in.at[0])
        cp_mem = pltpu.make_async_copy(mem_hbm, mem_v, sem_in.at[1])
        cp_wg = pltpu.make_async_copy(wg_hbm, wg_v, sem_in.at[2])
        cp_wu = pltpu.make_async_copy(wu_hbm, wu_v, sem_in.at[3])
        cp_wd = pltpu.make_async_copy(wd_hbm, wd_v, sem_in.at[4])

        cp_mem.start()
        cp_xd.start()
        cp_mem.wait()
        for cp in qkv_copies(0) + qkv_copies(1) + ox_copies(0):
            cp.start()

        lane_p = jax.lax.broadcasted_iota(jnp.int32, (1, 1, PW), 2)
        is_a3 = lane_p < DH

        def project(p, w0, w1):
            col = p * PW if isinstance(p, int) else pl.multiple_of(p * PW, 128)
            w = stage[p % NSLOT, w0 * PW:w1 * PW, :]
            sb = NSEG // PRB
            for b in range(PRB):
                y = jax.lax.dot_general(xd_v[b * sb * RD:(b + 1) * sb * RD, :], w, _NT,
                                        preferred_element_type=F32)
                y3 = y.reshape(sb, RD, (w1 - w0) * PW)
                for which in range(w0, w1):
                    yw = y3[:, :, (which - w0) * PW:(which - w0 + 1) * PW]
                    if which == 0:
                        qd[b * sb:(b + 1) * sb, :, pl.ds(col, PW)] = yw.astype(BF16)
                    else:
                        ya = jnp.where(is_a3, yw, 0.0)
                        yb = jnp.where(is_a3, 0.0, yw)
                        dst = kd2 if which == 1 else vd2
                        dst[b * sb:(b + 1) * sb, :, pl.ds(col, PW)] = pltpu.bitcast(
                            jnp.concatenate([ya, yb], axis=1).astype(BF16), jnp.uint32)
            wqkv[p, :, w0 * PW:w1 * PW] = pltpu.bitcast(w.T, jnp.uint32)

        def finish_ox(p):
            wo_v[p] = pltpu.bitcast(stage[p % NSLOT, 3 * PW:4 * PW, :], jnp.uint32)
            seg0 = p * SPP if isinstance(p, int) else pl.multiple_of(p * SPP, SPP)
            h_v[pl.ds(seg0, SPP), RD:SEG, :] = _ln(x_v[pl.ds(seg0, SPP), RD:SEG, :].astype(F32))

        cp_xd.wait()
        xd = xd_raw[...].astype(F32).reshape(ND, D)
        xd_v[...] = _ln(xd).astype(BF16)
        w_copy(0, 0).wait()
        for cp in qkv_copies(2) + ox_copies(1):
            cp.start()
        project(0, 0, 1)
        w_copy(0, 1).wait()
        w_copy(0, 2).wait()
        project(0, 1, 3)

        def pro_body(p, carry):
            for cp in qkv_copies(p) + ox_copies(p - 1):
                cp.wait()

            @pl.when(p + 2 < NP)
            def _():
                for cp in qkv_copies(p + 2):
                    cp.start()

            @pl.when(p + 1 < NP)
            def _():
                for cp in ox_copies(p + 1):
                    cp.start()

            project(p, 0, 3)
            finish_ox(p - 1)
            return carry

        jax.lax.fori_loop(1, NP, pro_body, 0)
        for cp in ox_copies(NP - 1):
            cp.wait()
        cp_wg.start()
        cp_wu.start()
        cp_wd.start()
        finish_ox(NP - 1)

        NK = 2 * (R1 + RD)
        row = jax.lax.broadcasted_iota(jnp.int32, (R1, NK), 0)
        lane = jax.lax.broadcasted_iota(jnp.int32, (R1, NK), 1)
        c_own_a = (lane < R1) | ((lane >= 2 * R1) & (lane < 2 * R1 + RD))
        c_own_b = jnp.logical_not(c_own_a)
        c_vis = (row < M) | (lane >= 2 * R1) | ((lane & (R1 - 1)) <= row)
        NKD = 2 * 2 * (M + RD)
        rowd = jax.lax.broadcasted_iota(jnp.int32, (2 * RD, NKD), 0)
        laned = jax.lax.broadcasted_iota(jnp.int32, (2 * RD, NKD), 1)
        same_seg = (rowd >= RD) == (laned >= NKD // 2)
        d_is_a = (laned & RD) == 0
        d_own_a = same_seg & d_is_a
        d_own_b = same_seg & jnp.logical_not(d_is_a)
        d_vis = ((laned & (2 * M)) == 0) | ((laned & (RD - 1)) <= (rowd & (RD - 1)))
        lane1 = jax.lax.broadcasted_iota(jnp.int32, (1, NKD), 1)
        lane2 = jax.lax.broadcasted_iota(jnp.int32, (1, PW), 1)
        is_a2 = lane2 < DH
        is_lo = jax.lax.broadcasted_iota(jnp.int32, (1, 128), 1) < DH - 128

        def seg_step(sd, s, half, m, xn, fill, erows, prog):
            l1 = jnp.concatenate([m, xn], axis=0).astype(BF16)

            def blockdiag(t, d2_ref, is_key, c0, c1):
                ta = jnp.where(is_a2, t, 0.0)
                tb = jnp.where(is_a2, 0.0, t)
                d2 = pltpu.bitcast(d2_ref[s, :, c0:c1], BF16)
                if is_key:
                    d2f = d2.astype(F32)
                    kf[half, 0:M, c0:c1] = t[0:M]
                    kf[half, M:M + RD, c0:c1] = d2f[0:RD] + d2f[RD:2 * RD]
                else:
                    vm2[half, :, c0:c1] = pltpu.bitcast(jnp.concatenate(
                        [ta[0:M], tb[0:M]], axis=0).astype(BF16), jnp.uint32)
                return jnp.concatenate([ta.astype(BF16), tb.astype(BF16), d2], axis=0)

            def stage_a(p):
                c0, c1 = p * PW, (p + 1) * PW
                y = jnp.dot(l1, pltpu.bitcast(wqkv[p], BF16), preferred_element_type=F32)
                qf = y[:, 0:PW].astype(BF16)
                kbd = blockdiag(y[:, PW:2 * PW], kd2, True, c0, c1)
                vbd = blockdiag(y[:, 2 * PW:3 * PW], vd2, False, c0, c1)
                return qf, kbd, vbd

            def stage_ae(p, pe):
                c0, c1 = p * PW, (p + 1) * PW
                ys, part = [], None
                for i in AE_ORDER:
                    ys.append((i, jnp.dot(l1, pltpu.bitcast(wqkv[p, :, i * PW:(i + 1) * PW], BF16),
                                          preferred_element_type=F32)))
                    e0 = pe * PW + len(ys) * 128 - 128
                    r0 = (len(ys) - 1) * 64
                    pi = jnp.dot(pltpu.bitcast(o_v[0:erows // 2, e0:e0 + 128], BF16),
                                 pltpu.bitcast(wo_v[pe, r0:r0 + 64, :], BF16),
                                 preferred_element_type=F32)
                    part = pi if part is None else part + pi
                ys = dict(ys)
                return (ys[0].astype(BF16), blockdiag(ys[1], kd2, True, c0, c1),
                        blockdiag(ys[2], vd2, False, c0, c1)), part

            def stage_b(qf, kbd):
                sc = jax.lax.dot_general(qf, kbd, _NT, preferred_element_type=F32) * scale
                return _pair_softmax(sc, c_vis, c_own_a, c_own_b)

            def stage_d(p, pm, vbd):
                c0, c1 = p * PW, (p + 1) * PW
                o_v[0:R1 // 2, c0:c1] = pltpu.bitcast(
                    jnp.dot(pm, vbd, preferred_element_type=F32).astype(BF16), jnp.uint32)

            def stage_e(p0, p1):
                c0, c1 = p0 * PW, p1 * PW
                wo = pltpu.bitcast(wo_v[p0:p1].reshape((p1 - p0) * PW // 2, D), BF16)
                return jnp.dot(pltpu.bitcast(o_v[0:erows // 2, c0:c1], BF16), wo,
                               preferred_element_type=F32)

            def stage_v(p):
                c0 = p * PW
                t0, t1, t2 = (slice(c0 + i * 128, c0 + (i + 1) * 128) for i in range(3))
                q = qd[s, :, c0:c0 + PW].astype(F32) * scale
                q0, q2 = q[:, 0:128], q[:, 256:384]
                q1a = jnp.where(is_lo, q[:, 128:256], 0.0)
                q1b = jnp.where(is_lo, 0.0, q[:, 128:256])
                sc = jnp.zeros((RD, NKD), F32)
                for jk in range(M + RD):
                    k1 = kf[half, jk:jk + 1, t1]
                    a = jnp.sum(q0 * kf[half, jk:jk + 1, t0] + q1a * k1, axis=1, keepdims=True)
                    b = jnp.sum(q2 * kf[half, jk:jk + 1, t2] + q1b * k1, axis=1, keepdims=True)
                    la = half * (NKD // 2) + (jk // M) * 2 * M + jk % M
                    sc = jnp.where(lane1 == la, a, jnp.where(lane1 == la + M, b, sc))
                sd.setdefault(p, []).append(sc)

            def stage_w(p):
                c0, c1 = p * PW, (p + 1) * PW
                pm = _pair_softmax(jnp.concatenate(sd[p], axis=0), d_vis, d_own_a, d_own_b)
                v = pltpu.bitcast(jnp.concatenate(
                    [vm2[0, :, c0:c1], vd2[s - 1, :, c0:c1],
                     vm2[1, :, c0:c1], vd2[s, :, c0:c1]], axis=0), BF16)
                o_v[R1 // 2:R1 // 2 + RD, c0:c1] = pltpu.bitcast(
                    jnp.dot(pm, v, preferred_element_type=F32).astype(BF16), jnp.uint32)

            abuf = {}
            pbuf = {}
            done = set()
            acc = None
            for tok in prog:
                op = tok[0]
                if op == "F":
                    if fill:
                        fill.pop(0)()
                    continue
                if op == "AE":
                    assert ("D", tok[2]) in done and ("W", tok[2]) in done
                    done.add(("A", tok[1]))
                    done.add(("E", tok[2], tok[2] + 1))
                    abuf[tok[1]], part = stage_ae(tok[1], tok[2])
                    acc = part if acc is None else acc + part
                    continue
                done.add(tok)
                if op == "A":
                    abuf[tok[1]] = stage_a(tok[1])
                elif op == "B":
                    pbuf[tok[1]] = stage_b(abuf[tok[1]][0], abuf[tok[1]][1])
                elif op == "D":
                    stage_d(tok[1], pbuf[tok[1]], abuf[tok[1]][2])
                elif op == "V":
                    assert ("A", tok[1]) in done
                    stage_v(tok[1])
                elif op == "W":
                    assert ("V", tok[1]) in done and half == 1
                    stage_w(tok[1])
                else:
                    assert all(("D", p) in done and (half == 0 or ("W", p) in done)
                               for p in range(tok[1], tok[2]))
                    part = stage_e(tok[1], tok[2])
                    acc = part if acc is None else acc + part
            assert all((o, p) in done for o in "ABDV" for p in range(NP))
            assert sorted(p for t in done if t[0] == "E" for p in range(t[1], t[2])) == list(range(NP))
            h_v[s, RD:SEG, :] = x_v[s, RD:SEG, :].astype(F32) + acc[M:R1]
            return acc

        def out_copy(j):
            s0 = j * 2 if isinstance(j, int) else pl.multiple_of(j * 2, 2)
            return pltpu.make_async_copy(
                out_v.at[pl.ds(s0, 2)], out_hbm.at[pl.ds(s0, 2)], sem_out.at[j])

        def main_body(j, m, first=False):
            s0 = 0 if first else pl.multiple_of(2 * j, 2)
            xn0 = h_v[s0, RD:SEG, :]
            xn1 = h_v[s0 + 1, RD:SEG, :]
            pieces = []
            if not first:
                s1 = pl.multiple_of((j - 1) * 2, 2)
                hb_v[...] = h_v[pl.ds(s1, 2)].reshape(FR, D)
                hn = _ln(hb_v[...]).astype(BF16)

                gbuf = {}

                def gate(c):
                    gbuf[c] = jnp.dot(hn, wg_v[:, c * FW:(c + 1) * FW], preferred_element_type=F32)

                def up(c):
                    u = jnp.dot(hn, wu_v[:, c * FW:(c + 1) * FW], preferred_element_type=F32)
                    g = gbuf[c]
                    act_v[:, c * FW:(c + 1) * FW] = pltpu.bitcast(
                        (g * jax.nn.sigmoid(g) * u).astype(BF16), jnp.uint32)

                def down(n, part):
                    n0, n1 = n * 128, (n + 1) * 128
                    f0, f1 = part * (F // DSPLIT), (part + 1) * (F // DSPLIT)
                    y = hb_v[:, n0:n1] + jnp.dot(pltpu.bitcast(act_v[:, f0:f1], BF16),
                                                 wd_v[f0:f1, n0:n1], preferred_element_type=F32)
                    if part < DSPLIT - 1:
                        hb_v[:, n0:n1] = y
                    else:
                        out_v[pl.ds(s1, 2), :, n0:n1] = y.astype(BF16).reshape(2, SEG, 128)

                for c in range(FC):
                    pieces += [functools.partial(gate, c), functools.partial(up, c)]
                for part in range(DSPLIT):
                    pieces += [functools.partial(down, n, part) for n in range(D // 128)]
            sd = {}
            acc = seg_step(sd, s0, 0, m, xn0, pieces, R1, PROG_A)
            acc = seg_step(sd, s0 + 1, 1, acc[0:M], xn1, pieces, R1 + 2 * RD, PROG_B)
            assert not pieces
            h_v[s0, 0:RD, :] = x_v[s0, 0:RD, :].astype(F32) + acc[R1:R1 + RD]
            h_v[s0 + 1, 0:RD, :] = x_v[s0 + 1, 0:RD, :].astype(F32) + acc[R1 + RD:R1 + 2 * RD]
            if not first:
                out_copy(j - 1).start()
            return acc[0:M]

        m1 = main_body(0, mem_v[...].astype(F32), first=True)
        cp_wg.wait()
        cp_wu.wait()
        cp_wd.wait()
        jax.lax.fori_loop(1, NJ, main_body, m1)

        sl = NSEG - 2
        h = h_v[sl:NSEG].reshape(FR, D)
        hn = _ln(h).astype(BF16)
        g = jnp.dot(hn, wg_v[...], preferred_element_type=F32)
        u = jnp.dot(hn, wu_v[...], preferred_element_type=F32)
        act = (g * jax.nn.sigmoid(g) * u).astype(BF16)
        y = h + jnp.dot(act, wd_v[...], preferred_element_type=F32)
        out_v[sl:NSEG] = y.astype(BF16).reshape(2, SEG, D)
        out_copy(NJ - 1).start()
        for j in range(NJ):
            out_copy(j).wait()

    scratch = [
        pltpu.VMEM((NSEG, SEG, D), BF16),
        pltpu.VMEM((M, D), BF16),
        pltpu.VMEM((NSLOT, 4 * PW, D), BF16),
        pltpu.VMEM((NP, D // 2, 3 * PW), jnp.uint32),
        pltpu.VMEM((NP, PW // 2, D), jnp.uint32),
        pltpu.VMEM((D, F), BF16),
        pltpu.VMEM((D, F), BF16),
        pltpu.VMEM((F, D), BF16),
        pltpu.VMEM((NSEG, RD, D), BF16),
        pltpu.VMEM((ND, D), BF16),
        pltpu.VMEM((NSEG, RD, H * DH), BF16),
        pltpu.VMEM((NSEG, RD, H * DH), jnp.uint32),
        pltpu.VMEM((NSEG, RD, H * DH), jnp.uint32),
        pltpu.VMEM((2, M + RD, H * DH), F32),
        pltpu.VMEM((2, M, H * DH), jnp.uint32),
        pltpu.VMEM((NSEG, SEG, D), F32),
        pltpu.VMEM((NSEG, SEG, D), BF16),
        pltpu.VMEM((R1 // 2 + RD, H * DH), jnp.uint32),
        pltpu.VMEM((FR, D), F32),
        pltpu.VMEM((FR // 2, F), jnp.uint32),
        pltpu.SemaphoreType.DMA((5,)),
        pltpu.SemaphoreType.DMA((NSLOT, 5)),
        pltpu.SemaphoreType.DMA((NJ,)),
    ]
    return kernel, scratch


@functools.partial(jax.jit, static_argnames=("seg",))
def _impl(A_x, A_mem0, A_Wq, A_Wk, A_Wv, A_Wo, B_w_gate, B_w_up, B_w_down, *, seg):
    B, S, D = A_x.shape
    _, H, DH = A_Wq.shape
    M = A_mem0.shape[1]
    F = B_w_gate.shape[1]
    assert B == 1 and S % seg == 0 and seg == 32 and M == 8
    nseg = S // seg

    kernel, scratch = _make_kernel(S, D, H, DH, M, seg, F)

    x3 = A_x.reshape(nseg, seg, D)
    mem = A_mem0.reshape(M, D)
    wqT = jnp.transpose(A_Wq, (1, 2, 0)).reshape(H * DH, D)
    wkT = jnp.transpose(A_Wk, (1, 2, 0)).reshape(H * DH, D)
    wvT = jnp.transpose(A_Wv, (1, 2, 0)).reshape(H * DH, D)
    wo = A_Wo.reshape(H * DH, D)

    out = pl.pallas_call(
        kernel,
        out_shape=jax.ShapeDtypeStruct((nseg, seg, D), A_x.dtype),
        in_specs=[pl.BlockSpec(memory_space=pl.ANY)] * 9,
        out_specs=pl.BlockSpec(memory_space=pl.ANY),
        scratch_shapes=scratch,
        compiler_params=pltpu.CompilerParams(vmem_limit_bytes=110 * 1024 * 1024, disable_bounds_checks=True, disable_semaphore_checks=True),
    )(x3, mem, wqT, wkT, wvT, wo, B_w_gate, B_w_up, B_w_down)
    return out.reshape(B, S, D)


def pallas_sequential_preLN__memory_aug_recurrent_mem_tr__swiglu_ffn__prompt_kernel(
    A_x,
    A_mem0,
    A_Wq,
    A_Wk,
    A_Wv,
    A_Wo,
    A_seg_len,
    B_x,
    B_w_gate,
    B_w_up,
    B_w_down,
):
    seg = A_seg_len if isinstance(A_seg_len, int) else 32
    return _impl(A_x, A_mem0, A_Wq, A_Wk, A_Wv, A_Wo, B_w_gate, B_w_up, B_w_down, seg=seg)
```

```python
import functools

import jax
import jax.numpy as jnp
import jax.experimental.pallas as pl
import jax.experimental.pallas.tpu as pltpu

F32 = jnp.float32
BF16 = jnp.bfloat16

_NT = (((1,), (1,)), ((), ()))
_NEG = -1000000000.0


def _ln(x):
    m = jnp.mean(x, axis=-1, keepdims=True)
    xc = x - m
    v = jnp.mean(xc * xc, axis=-1, keepdims=True)
    return xc * jax.lax.rsqrt(v + 1e-05)


def _pair_softmax(sc, visible, own_a, own_b):
    sc = jnp.where(visible, sc, _NEG)
    sa_ = jnp.where(own_a, sc, -jnp.inf)
    sb_ = jnp.where(own_b, sc, -jnp.inf)
    ma = jnp.max(sa_, axis=1, keepdims=True)
    mb = jnp.max(sb_, axis=1, keepdims=True)
    e = jnp.exp(jnp.where(own_a, sa_ - ma, sb_ - mb))
    da = jnp.sum(jnp.where(own_a, e, 0.0), axis=1, keepdims=True)
    db = jnp.sum(jnp.where(own_a, 0.0, e), axis=1, keepdims=True)
    return (e / jnp.where(own_a, da, db)).astype(BF16)


def _make_kernel(S, D, H, DH, M, SEG, F):
    NSEG = S // SEG
    NP = H // 2
    PW = 2 * DH
    RD = M
    RP = SEG - RD
    R1 = M + RP
    ND = NSEG * RD
    NSLOT = 4
    PRB = 4
    SPP = NSEG // NP
    NJ = NSEG // 2
    FW = 128
    FC = F // FW
    FR = 2 * SEG
    DSPLIT = 2
    LAGW = 4
    LAGE = 6
    FB_STEPS = (1, 2, 3, 4, 5, 7, 9, 11)
    AE_ORDER = (1, 0, 2)
    ESPLIT = 1

    def steps(second, LAGE=LAGE):
        prog = []
        for t in range(NP):
            if second and t >= LAGE and ESPLIT:
                prog.append(("AE", t, t - LAGE))
            else:
                prog.append(("A", t))
                if second and t >= LAGE:
                    prog.append(("E", t - LAGE, t - LAGE + 1))
            if t >= 1 and (not second or t in FB_STEPS):
                prog.append(("F",))
            if t >= 3:
                prog.append(("D", t - 3))
            if second and t >= LAGW:
                prog.append(("W", t - LAGW))
            if t >= 1:
                prog += [("B", t - 1), ("V", t - 1)]
        prog.append(("V", NP - 1))
        return prog

    F_ = ("F",)
    PROG_A = steps(False) + [("E", 0, 2), F_, ("D", 13), ("B", 15), ("E", 2, 5), ("D", 14), ("E", 5, 8), ("D", 15), ("E", 8, 16), F_, F_]
    PROG_B = steps(True) + [("E", 10, 11), ("W", 12), F_, ("D", 13), ("B", 15), ("E", 11, 12), ("W", 13), F_, F_, ("E", 12, 13), ("D", 14), ("W", 14), F_, F_, ("E", 13, 14), ("D", 15), ("W", 15), F_, F_, F_, ("E", 14, 16)]
    LAGE0 = 10
    PROG_B0 = steps(True, LAGE0) + [("E", 6, 7), ("W", 12), ("D", 13), ("B", 15), ("E", 7, 8), ("W", 13), ("E", 8, 10), ("D", 14), ("W", 14), ("E", 10, 12), ("D", 15), ("W", 15), ("E", 12, 16)]
    scale = float(DH) ** -0.5

    def kernel(x_hbm, mem_hbm, wq_hbm, wk_hbm, wv_hbm, wo_hbm, wg_hbm, wu_hbm, wd_hbm,
               out_hbm,
               x_v, mem_v, stage, wqkv, wo_v, wg_v, wu_v, wd_v,
               xd_raw, xd_v, qd, kd2, vd2, kf, vm2, hc_v, h_v, out_v, o_v, hb_v, act_v,
               sem_in, sem_stage, sem_out):
        w_hbm = (wq_hbm, wk_hbm, wv_hbm, wo_hbm)

        def w_copy(p, which):
            slot = p % NSLOT
            return pltpu.make_async_copy(
                w_hbm[which].at[pl.ds(p * PW, PW), :],
                stage.at[slot, pl.ds(which * PW, PW), :], sem_stage.at[slot, which])

        def qkv_copies(p):
            return [w_copy(p, which) for which in range(3)]

        def ox_copies(p):
            return [w_copy(p, 3), pltpu.make_async_copy(
                x_hbm.at[pl.ds(p * SPP, SPP)], x_v.at[pl.ds(p * SPP, SPP)],
                sem_stage.at[p % NSLOT, 4])]

        cp_xd = pltpu.make_async_copy(x_hbm.at[:, pl.ds(0, RD), :], xd_raw, sem_in.at[0])
        cp_mem = pltpu.make_async_copy(mem_hbm, mem_v, sem_in.at[1])
        cp_wg = pltpu.make_async_copy(wg_hbm, wg_v, sem_in.at[2])
        cp_wu = pltpu.make_async_copy(wu_hbm, wu_v, sem_in.at[3])
        cp_wd = pltpu.make_async_copy(wd_hbm, wd_v, sem_in.at[4])

        cp_mem.start()
        cp_xd.start()
        cp_mem.wait()
        for cp in qkv_copies(0) + qkv_copies(1) + ox_copies(0):
            cp.start()

        lane_p = jax.lax.broadcasted_iota(jnp.int32, (1, 1, PW), 2)
        is_a3 = lane_p < DH

        def project(p, w0, w1):
            col = p * PW if isinstance(p, int) else pl.multiple_of(p * PW, 128)
            w = stage[p % NSLOT, w0 * PW:w1 * PW, :]
            sb = NSEG // PRB
            for b in range(PRB):
                y = jax.lax.dot_general(xd_v[b * sb * RD:(b + 1) * sb * RD, :], w, _NT,
                                        preferred_element_type=F32)
                y3 = y.reshape(sb, RD, (w1 - w0) * PW)
                for which in range(w0, w1):
                    yw = y3[:, :, (which - w0) * PW:(which - w0 + 1) * PW]
                    if which == 0:
                        qd[b * sb:(b + 1) * sb, :, pl.ds(col, PW)] = yw.astype(BF16)
                    else:
                        ya = jnp.where(is_a3, yw, 0.0)
                        yb = jnp.where(is_a3, 0.0, yw)
                        dst = kd2 if which == 1 else vd2
                        dst[b * sb:(b + 1) * sb, :, pl.ds(col, PW)] = pltpu.bitcast(
                            jnp.concatenate([ya, yb], axis=1).astype(BF16), jnp.uint32)
            wqkv[p, :, w0 * PW:w1 * PW] = pltpu.bitcast(w.T, jnp.uint32)

        def finish_ox(p):
            wo_v[p] = pltpu.bitcast(stage[p % NSLOT, 3 * PW:4 * PW, :], jnp.uint32)
            seg0 = p * SPP if isinstance(p, int) else pl.multiple_of(p * SPP, SPP)
            h_v[pl.ds(seg0, SPP), RD:SEG, :] = _ln(x_v[pl.ds(seg0, SPP), RD:SEG, :].astype(F32))

        cp_xd.wait()
        xd = xd_raw[...].astype(F32).reshape(ND, D)
        xd_v[...] = _ln(xd).astype(BF16)
        w_copy(0, 0).wait()
        for cp in qkv_copies(2) + ox_copies(1):
            cp.start()
        project(0, 0, 1)
        w_copy(0, 1).wait()
        w_copy(0, 2).wait()
        project(0, 1, 3)

        def pro_body(p, carry):
            for cp in qkv_copies(p) + ox_copies(p - 1):
                cp.wait()

            @pl.when(p + 2 < NP)
            def _():
                for cp in qkv_copies(p + 2):
                    cp.start()

            @pl.when(p + 1 < NP)
            def _():
                for cp in ox_copies(p + 1):
                    cp.start()

            project(p, 0, 3)
            finish_ox(p - 1)
            return carry

        jax.lax.fori_loop(1, NP, pro_body, 0)
        for cp in ox_copies(NP - 1):
            cp.wait()
        cp_wg.start()
        cp_wu.start()
        cp_wd.start()
        finish_ox(NP - 1)

        NK = 2 * (R1 + RD)
        row = jax.lax.broadcasted_iota(jnp.int32, (R1, NK), 0)
        lane = jax.lax.broadcasted_iota(jnp.int32, (R1, NK), 1)
        c_own_a = (lane < R1) | ((lane >= 2 * R1) & (lane < 2 * R1 + RD))
        c_own_b = jnp.logical_not(c_own_a)
        c_vis = (row < M) | (lane >= 2 * R1) | ((lane & (R1 - 1)) <= row)
        NKD = 2 * 2 * (M + RD)
        rowd = jax.lax.broadcasted_iota(jnp.int32, (2 * RD, NKD), 0)
        laned = jax.lax.broadcasted_iota(jnp.int32, (2 * RD, NKD), 1)
        same_seg = (rowd >= RD) == (laned >= NKD // 2)
        d_is_a = (laned & RD) == 0
        d_own_a = same_seg & d_is_a
        d_own_b = same_seg & jnp.logical_not(d_is_a)
        d_vis = ((laned & (2 * M)) == 0) | ((laned & (RD - 1)) <= (rowd & (RD - 1)))
        lane1 = jax.lax.broadcasted_iota(jnp.int32, (1, NKD), 1)
        lane2 = jax.lax.broadcasted_iota(jnp.int32, (1, PW), 1)
        is_a2 = lane2 < DH
        is_lo = jax.lax.broadcasted_iota(jnp.int32, (1, 128), 1) < DH - 128

        def seg_step(sd, s, half, m, xn, fill, erows, prog):
            l1 = jnp.concatenate([m, xn], axis=0).astype(BF16)

            def blockdiag(t, d2_ref, is_key, c0, c1):
                ta = jnp.where(is_a2, t, 0.0)
                tb = jnp.where(is_a2, 0.0, t)
                d2u = d2_ref[s, :, c0:c1]
                d2 = pltpu.bitcast(d2u, BF16)
                if is_key:
                    d2f = d2.astype(F32)
                    kf[half, 0:M, c0:c1] = t[0:M]
                    kf[half, M:M + RD, c0:c1] = d2f[0:RD] + d2f[RD:2 * RD]
                else:
                    vm2[half, 0:M, c0:c1] = pltpu.bitcast(jnp.concatenate(
                        [ta[0:M], tb[0:M]], axis=0).astype(BF16), jnp.uint32)
                    vm2[half, M:M + RD, c0:c1] = d2u
                return jnp.concatenate([ta.astype(BF16), tb.astype(BF16), d2], axis=0)

            def stage_a(p):
                c0, c1 = p * PW, (p + 1) * PW
                y = jnp.dot(l1, pltpu.bitcast(wqkv[p], BF16), preferred_element_type=F32)
                qf = y[:, 0:PW].astype(BF16)
                kbd = blockdiag(y[:, PW:2 * PW], kd2, True, c0, c1)
                vbd = blockdiag(y[:, 2 * PW:3 * PW], vd2, False, c0, c1)
                return qf, kbd, vbd

            def stage_ae(p, pe):
                c0, c1 = p * PW, (p + 1) * PW
                ys, part = [], None
                for i in AE_ORDER:
                    ys.append((i, jnp.dot(l1, pltpu.bitcast(wqkv[p, :, i * PW:(i + 1) * PW], BF16),
                                          preferred_element_type=F32)))
                    e0 = pe * PW + len(ys) * 128 - 128
                    r0 = (len(ys) - 1) * 64
                    pi = jnp.dot(pltpu.bitcast(o_v[0:erows // 2, e0:e0 + 128], BF16),
                                 pltpu.bitcast(wo_v[pe, r0:r0 + 64, :], BF16),
                                 preferred_element_type=F32)
                    part = pi if part is None else part + pi
                ys = dict(ys)
                return (ys[0].astype(BF16), blockdiag(ys[1], kd2, True, c0, c1),
                        blockdiag(ys[2], vd2, False, c0, c1)), part

            def stage_b(qf, kbd):
                sc = jax.lax.dot_general(qf, kbd, _NT, preferred_element_type=F32) * scale
                return _pair_softmax(sc, c_vis, c_own_a, c_own_b)

            def stage_d(p, pm, vbd):
                c0, c1 = p * PW, (p + 1) * PW
                o_v[0:R1 // 2, c0:c1] = pltpu.bitcast(
                    jnp.dot(pm, vbd, preferred_element_type=F32).astype(BF16), jnp.uint32)

            def stage_e(p0, p1):
                c0, c1 = p0 * PW, p1 * PW
                wo = pltpu.bitcast(wo_v[p0:p1].reshape((p1 - p0) * PW // 2, D), BF16)
                return jnp.dot(pltpu.bitcast(o_v[0:erows // 2, c0:c1], BF16), wo,
                               preferred_element_type=F32)

            def stage_v(p):
                c0 = p * PW
                t0, t1, t2 = (slice(c0 + i * 128, c0 + (i + 1) * 128) for i in range(3))
                q = qd[s, :, c0:c0 + PW].astype(F32) * scale
                q0, q2 = q[:, 0:128], q[:, 256:384]
                q1a = jnp.where(is_lo, q[:, 128:256], 0.0)
                q1b = jnp.where(is_lo, 0.0, q[:, 128:256])
                sc = jnp.zeros((RD, NKD), F32)
                for jk in range(M + RD):
                    k1 = kf[half, jk:jk + 1, t1]
                    a = jnp.sum(q0 * kf[half, jk:jk + 1, t0] + q1a * k1, axis=1, keepdims=True)
                    b = jnp.sum(q2 * kf[half, jk:jk + 1, t2] + q1b * k1, axis=1, keepdims=True)
                    la = half * (NKD // 2) + (jk // M) * 2 * M + jk % M
                    sc = jnp.where(lane1 == la, a, jnp.where(lane1 == la + M, b, sc))
                sd.setdefault(p, []).append(sc)

            def stage_w(p):
                c0, c1 = p * PW, (p + 1) * PW
                pm = _pair_softmax(jnp.concatenate(sd[p], axis=0), d_vis, d_own_a, d_own_b)
                v = pltpu.bitcast(jnp.concatenate(
                    [vm2[0, :, c0:c1], vm2[1, :, c0:c1]], axis=0), BF16)
                o_v[R1 // 2:R1 // 2 + RD, c0:c1] = pltpu.bitcast(
                    jnp.dot(pm, v, preferred_element_type=F32).astype(BF16), jnp.uint32)

            abuf = {}
            pbuf = {}
            done = set()
            acc = None
            for tok in prog:
                op = tok[0]
                if op == "F":
                    if fill:
                        fill.pop(0)()
                    continue
                if op == "AE":
                    assert ("D", tok[2]) in done and ("W", tok[2]) in done
                    done.add(("A", tok[1]))
                    done.add(("E", tok[2], tok[2] + 1))
                    abuf[tok[1]], part = stage_ae(tok[1], tok[2])
                    acc = part if acc is None else acc + part
                    continue
                done.add(tok)
                if op == "A":
                    abuf[tok[1]] = stage_a(tok[1])
                elif op == "B":
                    pbuf[tok[1]] = stage_b(abuf[tok[1]][0], abuf[tok[1]][1])
                elif op == "D":
                    stage_d(tok[1], pbuf[tok[1]], abuf[tok[1]][2])
                elif op == "V":
                    assert ("A", tok[1]) in done
                    stage_v(tok[1])
                elif op == "W":
                    assert ("V", tok[1]) in done and half == 1
                    stage_w(tok[1])
                else:
                    assert all(("D", p) in done and (half == 0 or ("W", p) in done)
                               for p in range(tok[1], tok[2]))
                    part = stage_e(tok[1], tok[2])
                    acc = part if acc is None else acc + part
            assert all((o, p) in done for o in "ABDV" for p in range(NP))
            assert sorted(p for t in done if t[0] == "E" for p in range(t[1], t[2])) == list(range(NP))
            hc_v[half, RD:SEG, :] = x_v[s, RD:SEG, :].astype(F32) + acc[M:R1]
            return acc

        def out_copy(j):
            s0 = j * 2 if isinstance(j, int) else pl.multiple_of(j * 2, 2)
            return pltpu.make_async_copy(
                out_v.at[pl.ds(s0, 2)], out_hbm.at[pl.ds(s0, 2)], sem_out.at[j])

        def main_body(j, m, first=False):
            s0 = 0 if first else pl.multiple_of(2 * j, 2)
            xn0 = h_v[s0, RD:SEG, :]
            xn1 = h_v[s0 + 1, RD:SEG, :]
            pieces = []
            if not first:
                s1 = pl.multiple_of((j - 1) * 2, 2)
                hb_v[...] = hc_v[...].reshape(FR, D)
                hn = _ln(hb_v[...]).astype(BF16)

                gbuf = {}

                def gate(c):
                    gbuf[c] = jnp.dot(hn, wg_v[:, c * FW:(c + 1) * FW], preferred_element_type=F32)

                def up(c):
                    u = jnp.dot(hn, wu_v[:, c * FW:(c + 1) * FW], preferred_element_type=F32)
                    g = gbuf[c]
                    act_v[:, c * FW:(c + 1) * FW] = pltpu.bitcast(
                        (g * jax.nn.sigmoid(g) * u).astype(BF16), jnp.uint32)

                def down(n, part):
                    n0, n1 = n * 128, (n + 1) * 128
                    f0, f1 = part * (F // DSPLIT), (part + 1) * (F // DSPLIT)
                    y = hb_v[:, n0:n1] + jnp.dot(pltpu.bitcast(act_v[:, f0:f1], BF16),
                                                 wd_v[f0:f1, n0:n1], preferred_element_type=F32)
                    if part < DSPLIT - 1:
                        hb_v[:, n0:n1] = y
                    else:
                        out_v[pl.ds(s1, 2), :, n0:n1] = y.astype(BF16).reshape(2, SEG, 128)

                for c in range(FC):
                    pieces += [functools.partial(gate, c), functools.partial(up, c)]
                for part in range(DSPLIT):
                    pieces += [functools.partial(down, n, part) for n in range(D // 128)]
            sd = {}
            acc = seg_step(sd, s0, 0, m, xn0, pieces, R1, PROG_A)
            acc = seg_step(sd, s0 + 1, 1, acc[0:M], xn1, pieces, R1 + 2 * RD,
                           PROG_B0 if first else PROG_B)
            assert not pieces
            hc_v[0, 0:RD, :] = x_v[s0, 0:RD, :].astype(F32) + acc[R1:R1 + RD]
            hc_v[1, 0:RD, :] = x_v[s0 + 1, 0:RD, :].astype(F32) + acc[R1 + RD:R1 + 2 * RD]
            if not first:
                out_copy(j - 1).start()
            return acc[0:M]

        m1 = main_body(0, mem_v[...].astype(F32), first=True)
        cp_wg.wait()
        cp_wu.wait()
        cp_wd.wait()
        jax.lax.fori_loop(1, NJ, main_body, m1)

        sl = NSEG - 2
        h = hc_v[...].reshape(FR, D)
        hn = _ln(h).astype(BF16)
        g = jnp.dot(hn, wg_v[...], preferred_element_type=F32)
        u = jnp.dot(hn, wu_v[...], preferred_element_type=F32)
        act = (g * jax.nn.sigmoid(g) * u).astype(BF16)
        y = h + jnp.dot(act, wd_v[...], preferred_element_type=F32)
        out_v[sl:NSEG] = y.astype(BF16).reshape(2, SEG, D)
        out_copy(NJ - 1).start()
        for j in range(NJ):
            out_copy(j).wait()

    scratch = [
        pltpu.VMEM((NSEG, SEG, D), BF16),
        pltpu.VMEM((M, D), BF16),
        pltpu.VMEM((NSLOT, 4 * PW, D), BF16),
        pltpu.VMEM((NP, D // 2, 3 * PW), jnp.uint32),
        pltpu.VMEM((NP, PW // 2, D), jnp.uint32),
        pltpu.VMEM((D, F), BF16),
        pltpu.VMEM((D, F), BF16),
        pltpu.VMEM((F, D), BF16),
        pltpu.VMEM((NSEG, RD, D), BF16),
        pltpu.VMEM((ND, D), BF16),
        pltpu.VMEM((NSEG, RD, H * DH), BF16),
        pltpu.VMEM((NSEG, RD, H * DH), jnp.uint32),
        pltpu.VMEM((NSEG, RD, H * DH), jnp.uint32),
        pltpu.VMEM((2, M + RD, H * DH), F32),
        pltpu.VMEM((2, M + RD, H * DH), jnp.uint32),
        pltpu.VMEM((2, SEG, D), F32),
        pltpu.VMEM((NSEG, SEG, D), F32),
        pltpu.VMEM((NSEG, SEG, D), BF16),
        pltpu.VMEM((R1 // 2 + RD, H * DH), jnp.uint32),
        pltpu.VMEM((FR, D), F32),
        pltpu.VMEM((FR // 2, F), jnp.uint32),
        pltpu.SemaphoreType.DMA((5,)),
        pltpu.SemaphoreType.DMA((NSLOT, 5)),
        pltpu.SemaphoreType.DMA((NJ,)),
    ]
    return kernel, scratch


@functools.partial(jax.jit, static_argnames=("seg",))
def _impl(A_x, A_mem0, A_Wq, A_Wk, A_Wv, A_Wo, B_w_gate, B_w_up, B_w_down, *, seg):
    B, S, D = A_x.shape
    _, H, DH = A_Wq.shape
    M = A_mem0.shape[1]
    F = B_w_gate.shape[1]
    assert B == 1 and S % seg == 0 and seg == 32 and M == 8
    nseg = S // seg

    kernel, scratch = _make_kernel(S, D, H, DH, M, seg, F)

    x3 = A_x.reshape(nseg, seg, D)
    mem = A_mem0.reshape(M, D)
    wqT = jnp.transpose(A_Wq, (1, 2, 0)).reshape(H * DH, D)
    wkT = jnp.transpose(A_Wk, (1, 2, 0)).reshape(H * DH, D)
    wvT = jnp.transpose(A_Wv, (1, 2, 0)).reshape(H * DH, D)
    wo = A_Wo.reshape(H * DH, D)

    out = pl.pallas_call(
        kernel,
        out_shape=jax.ShapeDtypeStruct((nseg, seg, D), A_x.dtype),
        in_specs=[pl.BlockSpec(memory_space=pl.ANY)] * 9,
        out_specs=pl.BlockSpec(memory_space=pl.ANY),
        scratch_shapes=scratch,
        compiler_params=pltpu.CompilerParams(vmem_limit_bytes=110 * 1024 * 1024, disable_bounds_checks=True, disable_semaphore_checks=True),
    )(x3, mem, wqT, wkT, wvT, wo, B_w_gate, B_w_up, B_w_down)
    return out.reshape(B, S, D)


def pallas_sequential_preLN__memory_aug_recurrent_mem_tr__swiglu_ffn__prompt_kernel(
    A_x,
    A_mem0,
    A_Wq,
    A_Wk,
    A_Wv,
    A_Wo,
    A_seg_len,
    B_x,
    B_w_gate,
    B_w_up,
    B_w_down,
):
    seg = A_seg_len if isinstance(A_seg_len, int) else 32
    return _impl(A_x, A_mem0, A_Wq, A_Wk, A_Wv, A_Wo, B_w_gate, B_w_up, B_w_down, seg=seg)
```

```python
import functools

import jax
import jax.numpy as jnp
import jax.experimental.pallas as pl
import jax.experimental.pallas.tpu as pltpu

F32 = jnp.float32
BF16 = jnp.bfloat16

_NT = (((1,), (1,)), ((), ()))
_NEG = -1000000000.0


def _ln(x):
    m = jnp.mean(x, axis=-1, keepdims=True)
    xc = x - m
    v = jnp.mean(xc * xc, axis=-1, keepdims=True)
    return xc * jax.lax.rsqrt(v + 1e-05)


def _pair_softmax(sc, visible, own_a, own_b):
    sc = jnp.where(visible, sc, _NEG)
    sa_ = jnp.where(own_a, sc, -jnp.inf)
    sb_ = jnp.where(own_b, sc, -jnp.inf)
    ma = jnp.max(sa_, axis=1, keepdims=True)
    mb = jnp.max(sb_, axis=1, keepdims=True)
    e = jnp.exp(jnp.where(own_a, sa_ - ma, sb_ - mb))
    da = jnp.sum(jnp.where(own_a, e, 0.0), axis=1, keepdims=True)
    db = jnp.sum(jnp.where(own_a, 0.0, e), axis=1, keepdims=True)
    return (e / jnp.where(own_a, da, db)).astype(BF16)


def _make_kernel(S, D, H, DH, M, SEG, F):
    NSEG = S // SEG
    NP = H // 2
    PW = 2 * DH
    RD = M
    RP = SEG - RD
    R1 = M + RP
    ND = NSEG * RD
    NSLOT = 4
    PRB = 4
    SPP = NSEG // NP
    NJ = NSEG // 2
    FW = 128
    FC = F // FW
    FR = 2 * SEG
    DSPLIT = 2
    assert NP == 16 and PW == 3 * 128 and R1 == 32 and D % 128 == 0 and F % (DSPLIT * 128) == 0

    LAGW = 4
    FB_STEPS = (1, 2, 3, 4, 5, 7, 9, 11)
    AE_ORDER = (1, 0, 2)

    def steps(second, lag_e):
        prog = []
        for t in range(NP):
            if second and t >= lag_e:
                prog.append(("AE", t, t - lag_e))
            else:
                prog.append(("A", t))
            if t >= 1 and (not second or t in FB_STEPS):
                prog.append(("F",))
            if t >= 3:
                prog.append(("D", t - 3))
            if second and t >= LAGW:
                prog.append(("W", t - LAGW))
            if t >= 1:
                prog += [("B", t - 1), ("V", t - 1)]
        prog.append(("V", NP - 1))
        return prog

    F_ = ("F",)
    PROG_A = steps(False, NP) + [
        ("E", 0, 2), F_, ("D", 13), ("B", 15), ("E", 2, 5), ("D", 14), ("E", 5, 8), ("D", 15),
        ("E", 8, 16), F_, F_]
    PROG_B = steps(True, 6) + [
        ("E", 10, 11), ("W", 12), F_, ("D", 13), ("B", 15), ("E", 11, 12), ("W", 13), F_, F_,
        ("E", 12, 13), ("D", 14), ("W", 14), F_, F_, ("E", 13, 14), ("D", 15), ("W", 15),
        F_, F_, F_, ("E", 14, 16)]
    PROG_B0 = steps(True, 10) + [
        ("E", 6, 7), ("W", 12), ("D", 13), ("B", 15), ("E", 7, 8), ("W", 13), ("E", 8, 10),
        ("D", 14), ("W", 14), ("E", 10, 12), ("D", 15), ("W", 15), ("E", 12, 16)]
    scale = float(DH) ** -0.5

    def kernel(x_hbm, mem_hbm, wq_hbm, wk_hbm, wv_hbm, wo_hbm, wg_hbm, wu_hbm, wd_hbm,
               out_hbm,
               x_v, mem_v, stage, wqkv, wo_v, wg_v, wu_v, wd_v,
               xd_raw, xd_v, qd, kd2, vd2, kf, vm2, hc_v, h_v, out_v, o_v, hb_v, act_v,
               sem_in, sem_stage, sem_out):
        w_hbm = (wq_hbm, wk_hbm, wv_hbm, wo_hbm)

        def w_copy(p, which):
            slot = p % NSLOT
            return pltpu.make_async_copy(
                w_hbm[which].at[pl.ds(p * PW, PW), :],
                stage.at[slot, pl.ds(which * PW, PW), :], sem_stage.at[slot * 5 + which])

        def qkv_copies(p):
            return [w_copy(p, which) for which in range(3)]

        def ox_copies(p):
            return [w_copy(p, 3), pltpu.make_async_copy(
                x_hbm.at[pl.ds(p * SPP, SPP)], x_v.at[pl.ds(p * SPP, SPP)],
                sem_stage.at[(p % NSLOT) * 5 + 4])]

        cp_xd = pltpu.make_async_copy(x_hbm.at[:, pl.ds(0, RD), :], xd_raw, sem_in.at[0])
        cp_mem = pltpu.make_async_copy(mem_hbm, mem_v, sem_in.at[1])
        cp_wg = pltpu.make_async_copy(wg_hbm, wg_v, sem_in.at[2])
        cp_wu = pltpu.make_async_copy(wu_hbm, wu_v, sem_in.at[3])
        cp_wd = pltpu.make_async_copy(wd_hbm, wd_v, sem_in.at[4])

        cp_mem.start()
        cp_xd.start()
        cp_mem.wait()
        for cp in qkv_copies(0) + qkv_copies(1) + ox_copies(0):
            cp.start()

        lane_p = jax.lax.broadcasted_iota(jnp.int32, (1, 1, PW), 2)
        is_a3 = lane_p < DH

        def project(p, w0, w1):
            col = p * PW if isinstance(p, int) else pl.multiple_of(p * PW, 128)
            w = stage[p % NSLOT, w0 * PW:w1 * PW, :]
            sb = NSEG // PRB
            for b in range(PRB):
                y = jax.lax.dot_general(xd_v[b * sb * RD:(b + 1) * sb * RD, :], w, _NT,
                                        preferred_element_type=F32)
                y3 = y.reshape(sb, RD, (w1 - w0) * PW)
                for which in range(w0, w1):
                    yw = y3[:, :, (which - w0) * PW:(which - w0 + 1) * PW]
                    if which == 0:
                        qd[b * sb:(b + 1) * sb, :, pl.ds(col, PW)] = yw.astype(BF16)
                    else:
                        ya = jnp.where(is_a3, yw, 0.0)
                        yb = jnp.where(is_a3, 0.0, yw)
                        dst = kd2 if which == 1 else vd2
                        dst[b * sb:(b + 1) * sb, :, pl.ds(col, PW)] = pltpu.bitcast(
                            jnp.concatenate([ya, yb], axis=1).astype(BF16), jnp.uint32)
            wqkv[p, :, w0 * PW:w1 * PW] = pltpu.bitcast(w.T, jnp.uint32)

        def finish_ox(p):
            wo_v[p] = pltpu.bitcast(stage[p % NSLOT, 3 * PW:4 * PW, :], jnp.uint32)
            seg0 = p * SPP if isinstance(p, int) else pl.multiple_of(p * SPP, SPP)
            h_v[pl.ds(seg0, SPP), RD:SEG, :] = _ln(x_v[pl.ds(seg0, SPP), RD:SEG, :].astype(F32))

        cp_xd.wait()
        xd = xd_raw[...].astype(F32).reshape(ND, D)
        xd_v[...] = _ln(xd).astype(BF16)
        w_copy(0, 0).wait()
        for cp in qkv_copies(2) + ox_copies(1):
            cp.start()
        project(0, 0, 1)
        w_copy(0, 1).wait()
        w_copy(0, 2).wait()
        project(0, 1, 3)

        def pro_body(p, carry):
            for cp in qkv_copies(p) + ox_copies(p - 1):
                cp.wait()

            @pl.when(p + 2 < NP)
            def _():
                for cp in qkv_copies(p + 2):
                    cp.start()

            @pl.when(p + 1 < NP)
            def _():
                for cp in ox_copies(p + 1):
                    cp.start()

            project(p, 0, 3)
            finish_ox(p - 1)
            return carry

        jax.lax.fori_loop(1, NP, pro_body, 0)
        for cp in ox_copies(NP - 1):
            cp.wait()
        cp_wg.start()
        cp_wu.start()
        cp_wd.start()
        finish_ox(NP - 1)

        NK = 2 * (R1 + RD)
        row = jax.lax.broadcasted_iota(jnp.int32, (R1, NK), 0)
        lane = jax.lax.broadcasted_iota(jnp.int32, (R1, NK), 1)
        c_own_a = (lane < R1) | ((lane >= 2 * R1) & (lane < 2 * R1 + RD))
        c_own_b = jnp.logical_not(c_own_a)
        c_vis = (row < M) | (lane >= 2 * R1) | ((lane & (R1 - 1)) <= row)
        NKD = 2 * 2 * (M + RD)
        rowd = jax.lax.broadcasted_iota(jnp.int32, (2 * RD, NKD), 0)
        laned = jax.lax.broadcasted_iota(jnp.int32, (2 * RD, NKD), 1)
        same_seg = (rowd >= RD) == (laned >= NKD // 2)
        d_is_a = (laned & RD) == 0
        d_own_a = same_seg & d_is_a
        d_own_b = same_seg & jnp.logical_not(d_is_a)
        d_vis = ((laned & (2 * M)) == 0) | ((laned & (RD - 1)) <= (rowd & (RD - 1)))
        lane1 = jax.lax.broadcasted_iota(jnp.int32, (1, NKD), 1)
        lane2 = jax.lax.broadcasted_iota(jnp.int32, (1, PW), 1)
        is_a2 = lane2 < DH
        is_lo = jax.lax.broadcasted_iota(jnp.int32, (1, 128), 1) < DH - 128

        def seg_step(sd, s, half, m, xn, fill, erows, prog):
            l1 = jnp.concatenate([m, xn], axis=0).astype(BF16)

            def blockdiag(t, d2_ref, is_key, c0, c1):
                ta = jnp.where(is_a2, t, 0.0)
                tb = jnp.where(is_a2, 0.0, t)
                d2u = d2_ref[s, :, c0:c1]
                d2 = pltpu.bitcast(d2u, BF16)
                if is_key:
                    d2f = d2.astype(F32)
                    kf[half, 0:M, c0:c1] = t[0:M]
                    kf[half, M:M + RD, c0:c1] = d2f[0:RD] + d2f[RD:2 * RD]
                else:
                    vm2[half, 0:M, c0:c1] = pltpu.bitcast(jnp.concatenate(
                        [ta[0:M], tb[0:M]], axis=0).astype(BF16), jnp.uint32)
                    vm2[half, M:M + RD, c0:c1] = d2u
                return jnp.concatenate([ta.astype(BF16), tb.astype(BF16), d2], axis=0)

            def stage_a(p):
                c0, c1 = p * PW, (p + 1) * PW
                y = jnp.dot(l1, pltpu.bitcast(wqkv[p], BF16), preferred_element_type=F32)
                qf = y[:, 0:PW].astype(BF16)
                kbd = blockdiag(y[:, PW:2 * PW], kd2, True, c0, c1)
                vbd = blockdiag(y[:, 2 * PW:3 * PW], vd2, False, c0, c1)
                return qf, kbd, vbd

            def stage_ae(p, pe):
                c0, c1 = p * PW, (p + 1) * PW
                ys, part = [], None
                for i in AE_ORDER:
                    ys.append((i, jnp.dot(l1, pltpu.bitcast(wqkv[p, :, i * PW:(i + 1) * PW], BF16),
                                          preferred_element_type=F32)))
                    e0 = pe * PW + len(ys) * 128 - 128
                    r0 = (len(ys) - 1) * 64
                    pi = jnp.dot(pltpu.bitcast(o_v[0:erows // 2, e0:e0 + 128], BF16),
                                 pltpu.bitcast(wo_v[pe, r0:r0 + 64, :], BF16),
                                 preferred_element_type=F32)
                    part = pi if part is None else part + pi
                ys = dict(ys)
                return (ys[0].astype(BF16), blockdiag(ys[1], kd2, True, c0, c1),
                        blockdiag(ys[2], vd2, False, c0, c1)), part

            def stage_b(qf, kbd):
                sc = jax.lax.dot_general(qf, kbd, _NT, preferred_element_type=F32) * scale
                return _pair_softmax(sc, c_vis, c_own_a, c_own_b)

            def stage_d(p, pm, vbd):
                c0, c1 = p * PW, (p + 1) * PW
                o_v[0:R1 // 2, c0:c1] = pltpu.bitcast(
                    jnp.dot(pm, vbd, preferred_element_type=F32).astype(BF16), jnp.uint32)

            def stage_e(p0, p1):
                c0, c1 = p0 * PW, p1 * PW
                wo = pltpu.bitcast(wo_v[p0:p1].reshape((p1 - p0) * PW // 2, D), BF16)
                return jnp.dot(pltpu.bitcast(o_v[0:erows // 2, c0:c1], BF16), wo,
                               preferred_element_type=F32)

            def stage_v(p):
                c0 = p * PW
                t0, t1, t2 = (slice(c0 + i * 128, c0 + (i + 1) * 128) for i in range(3))
                q = qd[s, :, c0:c0 + PW].astype(F32) * scale
                q0, q2 = q[:, 0:128], q[:, 256:384]
                q1a = jnp.where(is_lo, q[:, 128:256], 0.0)
                q1b = jnp.where(is_lo, 0.0, q[:, 128:256])
                sc = jnp.zeros((RD, NKD), F32)
                for jk in range(M + RD):
                    k1 = kf[half, jk:jk + 1, t1]
                    a = jnp.sum(q0 * kf[half, jk:jk + 1, t0] + q1a * k1, axis=1, keepdims=True)
                    b = jnp.sum(q2 * kf[half, jk:jk + 1, t2] + q1b * k1, axis=1, keepdims=True)
                    la = half * (NKD // 2) + (jk // M) * 2 * M + jk % M
                    sc = jnp.where(lane1 == la, a, jnp.where(lane1 == la + M, b, sc))
                sd.setdefault(p, []).append(sc)

            def stage_w(p):
                c0, c1 = p * PW, (p + 1) * PW
                pm = _pair_softmax(jnp.concatenate(sd[p], axis=0), d_vis, d_own_a, d_own_b)
                v = pltpu.bitcast(jnp.concatenate(
                    [vm2[0, :, c0:c1], vm2[1, :, c0:c1]], axis=0), BF16)
                o_v[R1 // 2:R1 // 2 + RD, c0:c1] = pltpu.bitcast(
                    jnp.dot(pm, v, preferred_element_type=F32).astype(BF16), jnp.uint32)

            abuf = {}
            pbuf = {}
            done = set()
            acc = None
            for tok in prog:
                op = tok[0]
                if op == "F":
                    if fill:
                        fill.pop(0)()
                    continue
                if op == "AE":
                    assert ("D", tok[2]) in done and ("W", tok[2]) in done
                    done.add(("A", tok[1]))
                    done.add(("E", tok[2], tok[2] + 1))
                    abuf[tok[1]], part = stage_ae(tok[1], tok[2])
                    acc = part if acc is None else acc + part
                    continue
                done.add(tok)
                if op == "A":
                    abuf[tok[1]] = stage_a(tok[1])
                elif op == "B":
                    pbuf[tok[1]] = stage_b(abuf[tok[1]][0], abuf[tok[1]][1])
                elif op == "D":
                    stage_d(tok[1], pbuf[tok[1]], abuf[tok[1]][2])
                elif op == "V":
                    assert ("A", tok[1]) in done
                    stage_v(tok[1])
                elif op == "W":
                    assert ("V", tok[1]) in done and half == 1
                    stage_w(tok[1])
                else:
                    assert all(("D", p) in done and (half == 0 or ("W", p) in done)
                               for p in range(tok[1], tok[2]))
                    part = stage_e(tok[1], tok[2])
                    acc = part if acc is None else acc + part
            assert all((o, p) in done for o in "ABDV" for p in range(NP))
            assert sorted(p for t in done if t[0] == "E" for p in range(t[1], t[2])) == list(range(NP))
            hc_v[half, RD:SEG, :] = x_v[s, RD:SEG, :].astype(F32) + acc[M:R1]
            return acc

        def out_copy(j):
            s0 = j * 2 if isinstance(j, int) else pl.multiple_of(j * 2, 2)
            return pltpu.make_async_copy(
                out_v.at[pl.ds(s0, 2)], out_hbm.at[pl.ds(s0, 2)], sem_out.at[j])

        def main_body(j, m, first=False):
            s0 = 0 if first else pl.multiple_of(2 * j, 2)
            xn0 = h_v[s0, RD:SEG, :]
            xn1 = h_v[s0 + 1, RD:SEG, :]
            pieces = []
            if not first:
                s1 = pl.multiple_of((j - 1) * 2, 2)
                hb_v[...] = hc_v[...].reshape(FR, D)
                hn = _ln(hb_v[...]).astype(BF16)

                gbuf = {}

                def gate(c):
                    gbuf[c] = jnp.dot(hn, wg_v[:, c * FW:(c + 1) * FW], preferred_element_type=F32)

                def up(c):
                    u = jnp.dot(hn, wu_v[:, c * FW:(c + 1) * FW], preferred_element_type=F32)
                    g = gbuf[c]
                    act_v[:, c * FW:(c + 1) * FW] = pltpu.bitcast(
                        (g * jax.nn.sigmoid(g) * u).astype(BF16), jnp.uint32)

                def down(n, part):
                    n0, n1 = n * 128, (n + 1) * 128
                    f0, f1 = part * (F // DSPLIT), (part + 1) * (F // DSPLIT)
                    y = hb_v[:, n0:n1] + jnp.dot(pltpu.bitcast(act_v[:, f0:f1], BF16),
                                                 wd_v[f0:f1, n0:n1], preferred_element_type=F32)
                    if part < DSPLIT - 1:
                        hb_v[:, n0:n1] = y
                    else:
                        out_v[pl.ds(s1, 2), :, n0:n1] = y.astype(BF16).reshape(2, SEG, 128)

                for c in range(FC):
                    pieces += [functools.partial(gate, c), functools.partial(up, c)]
                for part in range(DSPLIT):
                    pieces += [functools.partial(down, n, part) for n in range(D // 128)]
            sd = {}
            acc = seg_step(sd, s0, 0, m, xn0, pieces, R1, PROG_A)
            acc = seg_step(sd, s0 + 1, 1, acc[0:M], xn1, pieces, R1 + 2 * RD,
                           PROG_B0 if first else PROG_B)
            assert not pieces
            hc_v[0, 0:RD, :] = x_v[s0, 0:RD, :].astype(F32) + acc[R1:R1 + RD]
            hc_v[1, 0:RD, :] = x_v[s0 + 1, 0:RD, :].astype(F32) + acc[R1 + RD:R1 + 2 * RD]
            if not first:
                out_copy(j - 1).start()
            return acc[0:M]

        m1 = main_body(0, mem_v[...].astype(F32), first=True)
        cp_wg.wait()
        cp_wu.wait()
        cp_wd.wait()
        jax.lax.fori_loop(1, NJ, main_body, m1)

        sl = NSEG - 2
        h = hc_v[...].reshape(FR, D)
        hn = _ln(h).astype(BF16)
        g = jnp.dot(hn, wg_v[...], preferred_element_type=F32)
        u = jnp.dot(hn, wu_v[...], preferred_element_type=F32)
        act = (g * jax.nn.sigmoid(g) * u).astype(BF16)
        y = h + jnp.dot(act, wd_v[...], preferred_element_type=F32)
        out_v[sl:NSEG] = y.astype(BF16).reshape(2, SEG, D)
        out_copy(NJ - 1).start()
        for j in range(NJ):
            out_copy(j).wait()

    scratch = [
        pltpu.VMEM((NSEG, SEG, D), BF16),
        pltpu.VMEM((M, D), BF16),
        pltpu.VMEM((NSLOT, 4 * PW, D), BF16),
        pltpu.VMEM((NP, D // 2, 3 * PW), jnp.uint32),
        pltpu.VMEM((NP, PW // 2, D), jnp.uint32),
        pltpu.VMEM((D, F), BF16),
        pltpu.VMEM((D, F), BF16),
        pltpu.VMEM((F, D), BF16),
        pltpu.VMEM((NSEG, RD, D), BF16),
        pltpu.VMEM((ND, D), BF16),
        pltpu.VMEM((NSEG, RD, H * DH), BF16),
        pltpu.VMEM((NSEG, RD, H * DH), jnp.uint32),
        pltpu.VMEM((NSEG, RD, H * DH), jnp.uint32),
        pltpu.VMEM((2, M + RD, H * DH), F32),
        pltpu.VMEM((2, M + RD, H * DH), jnp.uint32),
        pltpu.VMEM((2, SEG, D), F32),
        pltpu.VMEM((NSEG, SEG, D), F32),
        pltpu.VMEM((NSEG, SEG, D), BF16),
        pltpu.VMEM((R1 // 2 + RD, H * DH), jnp.uint32),
        pltpu.VMEM((FR, D), F32),
        pltpu.VMEM((FR // 2, F), jnp.uint32),
        pltpu.SemaphoreType.DMA((5,)),
        pltpu.SemaphoreType.DMA((NSLOT * 5,)),
        pltpu.SemaphoreType.DMA((NJ,)),
    ]
    return kernel, scratch


@functools.partial(jax.jit, static_argnames=("seg",))
def _impl(A_x, A_mem0, A_Wq, A_Wk, A_Wv, A_Wo, B_w_gate, B_w_up, B_w_down, *, seg):
    B, S, D = A_x.shape
    _, H, DH = A_Wq.shape
    M = A_mem0.shape[1]
    F = B_w_gate.shape[1]
    assert B == 1 and S % seg == 0 and seg == 32 and M == 8
    nseg = S // seg

    kernel, scratch = _make_kernel(S, D, H, DH, M, seg, F)

    x3 = A_x.reshape(nseg, seg, D)
    mem = A_mem0.reshape(M, D)
    wqT = jnp.transpose(A_Wq, (1, 2, 0)).reshape(H * DH, D)
    wkT = jnp.transpose(A_Wk, (1, 2, 0)).reshape(H * DH, D)
    wvT = jnp.transpose(A_Wv, (1, 2, 0)).reshape(H * DH, D)
    wo = A_Wo.reshape(H * DH, D)

    out = pl.pallas_call(
        kernel,
        out_shape=jax.ShapeDtypeStruct((nseg, seg, D), A_x.dtype),
        in_specs=[pl.BlockSpec(memory_space=pl.ANY)] * 9,
        out_specs=pl.BlockSpec(memory_space=pl.ANY),
        scratch_shapes=scratch,
        compiler_params=pltpu.CompilerParams(
            vmem_limit_bytes=110 * 1024 * 1024,
            disable_bounds_checks=True,
            disable_semaphore_checks=True,
        ),
    )(x3, mem, wqT, wkT, wvT, wo, B_w_gate, B_w_up, B_w_down)
    return out.reshape(B, S, D)


def pallas_sequential_preLN__memory_aug_recurrent_mem_tr__swiglu_ffn__prompt_kernel(
    A_x,
    A_mem0,
    A_Wq,
    A_Wk,
    A_Wv,
    A_Wo,
    A_seg_len,
    B_x,
    B_w_gate,
    B_w_up,
    B_w_down,
):
    seg = A_seg_len if isinstance(A_seg_len, int) else 32
    return _impl(A_x, A_mem0, A_Wq, A_Wk, A_Wv, A_Wo, B_w_gate, B_w_up, B_w_down, seg=seg)
```
